```python
import jax
import jax.numpy as jnp

def _softmax(x, axis=-1):
    return jax.nn.softmax(x, axis=axis)

def _gelu(x):
    return jax.nn.gelu(x, approximate=True)

def _silu(x):
    return jax.nn.silu(x)

def _sigmoid(x):
    return jax.nn.sigmoid(x)

def _layernorm(x, axis=-1, eps=1e-05):
    m = jnp.mean(x, axis=axis, keepdims=True)
    v = jnp.var(x, axis=axis, keepdims=True)
    return (x - m) / jnp.sqrt(v + eps)

def _scatter_add(tgt, idx, src, axis=0):
    return tgt.at[idx].add(src)

def _segment_sum(src, seg, n):
    return jax.ops.segment_sum(src, seg, n)

class _Rng:

    def __init__(self, key):
        self._k = key

    def _next(self):
        self._k, sub = jax.random.split(self._k)
        return sub

    def normal(self, shape):
        return jax.random.normal(self._next(), shape, dtype=jnp.bfloat16)

    def randint(self, lo, hi, shape):
        return jax.random.randint(self._next(), shape, lo, hi, dtype=jnp.int32)

    def uniform(self, shape, lo=0.0, hi=1.0):
        return jax.random.uniform(self._next(), shape, jnp.bfloat16, lo, hi)

    def permutation(self, n):
        return jax.random.permutation(self._next(), n)
kernel_name = 'interleave_layers__memory_aug_infini_attn__mixer_s_mlp__prompt'

def setup_inputs():
    _rng = _Rng(jax.random.key(int.from_bytes(__import__("os").urandom(4), "little")))
    _w = lambda a: (lambda t: t.astype(jnp.bfloat16) if jnp.issubdtype(t.dtype, jnp.floating) else t)(jnp.asarray(a))

    def _A_setup():
        B, S, D, H = (1, 2048, 1024, 32)
        N = 4
        L = max(1, S // N)
        sc = D ** (-0.5)
        return {'x': _w((lambda *s: _rng.normal(s) * 0.05)(B, N * L, D)), 'wq': _w((lambda *s: _rng.normal(s) * 0.05)(D, D) * sc), 'wk': _w((lambda *s: _rng.normal(s) * 0.05)(D, D) * sc), 'wv': _w((lambda *s: _rng.normal(s) * 0.05)(D, D) * sc), 'wo': _w((lambda *s: _rng.normal(s) * 0.05)(D, D) * sc), 'beta': _w((lambda *s: _rng.normal(s) * 0.05)(H))}
    _A_in = _A_setup()

    def _B_setup():
        B, S, D, F = (1, 2048, 1024, 3584)
        return {'x': _w((lambda *s: _rng.normal(s) * 0.05)(B, S, D)), 'w1': _w((lambda *s: _rng.normal(s) * 0.05)(D, D) * D ** (-0.5)), 'w2': _w((lambda *s: _rng.normal(s) * 0.05)(D, D) * D ** (-0.5)), 'w3': _w((lambda *s: _rng.normal(s) * 0.05)(D, F) * D ** (-0.5)), 'w4': _w((lambda *s: _rng.normal(s) * 0.05)(F, D) * F ** (-0.5))}
    _B_in = _B_setup()
    return {'A_x': _A_in['x'], 'A_wq': _A_in['wq'], 'A_wk': _A_in['wk'], 'A_wv': _A_in['wv'], 'A_wo': _A_in['wo'], 'A_beta': _A_in['beta'], 'B_x': _B_in['x'], 'B_w1': _B_in['w1'], 'B_w2': _B_in['w2'], 'B_w3': _B_in['w3'], 'B_w4': _B_in['w4']}

def reference(A_x, A_wq, A_wk, A_wv, A_wo, A_beta, B_x, B_w1, B_w2, B_w3, B_w4):

    def _A_ref(x, wq, wk, wv, wo, beta):
        B, S, D = x.shape
        H = 32
        Dh = D // H
        N = 4
        L = S // N
        q = (lambda x, *d: x.transpose(*d))((x @ wq).reshape(B, S, H, Dh), 0, 2, 1, 3).reshape(B, H, N, L, Dh)
        k = (lambda x, *d: x.transpose(*d))((x @ wk).reshape(B, S, H, Dh), 0, 2, 1, 3).reshape(B, H, N, L, Dh)
        v = (lambda x, *d: x.transpose(*d))((x @ wv).reshape(B, S, H, Dh), 0, 2, 1, 3).reshape(B, H, N, L, Dh)
        phi = lambda t: jnp.where(t > 0, t + 1.0, jnp.exp(t))
        scale = Dh ** (-0.5)
        ar = jnp.arange(L)
        mask = (lambda x, dt: x.astype(dt))(ar[:, None] < ar[None, :], x.dtype) * -1000000000.0
        g = _sigmoid(beta).reshape(1, H, 1, 1)
        M = jnp.einsum('bhd,bhe->bhde', q[:, :, 0, 0, :] * 0.0, q[:, :, 0, 0, :] * 0.0)
        z = q[:, :, 0, 0, :] * 0.0
        outs = []
        for s in range(N):
            qs, ks, vs = (q[:, :, s].copy(), k[:, :, s].copy(), v[:, :, s].copy())
            logits = jnp.einsum('bhqd,bhkd->bhqk', qs, ks) * scale + mask
            p = _softmax(logits, axis=-1)
            a_dot = jnp.einsum('bhqk,bhkd->bhqd', p, vs)
            pq = phi(qs)
            num = jnp.einsum('bhld,bhde->bhle', pq, M)
            den = jnp.einsum('bhld,bhd->bhl', pq, z)[..., None] + 1e-06
            a_mem = num / den
            o = g * a_mem + (1.0 - g) * a_dot
            outs.append(o)
            pk = phi(ks)
            M = M + jnp.einsum('bhld,bhle->bhde', pk, vs)
            z = z + jnp.einsum('bhld->bhd', pk)
        o = (lambda x, *d: x.transpose(*d))(jnp.stack(outs, 2).reshape(B, H, S, Dh), 0, 2, 1, 3).reshape(B, S, D)
        return o @ wo

    def _B_ref(x, w1, w2, w3, w4):
        B, S, D = x.shape
        h = _gelu(_layernorm(x, axis=-1) @ w1)
        c = D // 4
        g0 = jnp.pad(h[:, :, 0 * c:1 * c], ((0, 0), (1, 0), (0, 0)))[:, :S, :]
        g1 = jnp.pad(h[:, :, 1 * c:2 * c], ((0, 0), (0, 1), (0, 0)))[:, 1:, :]
        g2 = jnp.pad(h[:, :, 2 * c:3 * c], ((0, 0), (2, 0), (0, 0)))[:, :S, :]
        g3 = jnp.pad(h[:, :, 3 * c:], ((0, 0), (0, 2), (0, 0)))[:, 2:, :]
        hs = jnp.concatenate([g0, g1, g2, g3], axis=-1) @ w2
        x1 = x + hs
        h2 = _gelu(_layernorm(x1, axis=-1) @ w3) @ w4
        return x1 + h2
    x = A_x
    x = x + _A_ref(_layernorm(x, axis=-1), A_wq, A_wk, A_wv, A_wo, A_beta)
    x = x + _B_ref(_layernorm(x, axis=-1), B_w1, B_w2, B_w3, B_w4)
    x = x + _A_ref(_layernorm(x, axis=-1), A_wq, A_wk, A_wv, A_wo, A_beta)
    x = x + _B_ref(_layernorm(x, axis=-1), B_w1, B_w2, B_w3, B_w4)
    return x
```

```python
import functools

import numpy as np
import jax
import jax.numpy as jnp
from jax import lax
import jax.experimental.pallas as pl
import jax.experimental.pallas.tpu as pltpu

S, D, H, DH, NSEG, L, F = 2048, 1024, 32, 32, 4, 512, 3584
NG = D // 128
BF, F32 = jnp.bfloat16, jnp.float32
NT = (((1,), (1,)), ((), ()))
EPS = 1e-5
LOG2E = float(np.log2(np.e))
QSCALE = float(DH ** -0.5) * LOG2E
GC = float(np.sqrt(2.0 / np.pi))
HPAD = 8
VR = 144


def _ln(x):
    m = jnp.mean(x, axis=-1, keepdims=True)
    xc = x - m
    v = jnp.mean(xc * xc, axis=-1, keepdims=True)
    return xc * lax.rsqrt(v + EPS)


def _gelu(x):
    return 0.5 * x * (1.0 + jnp.tanh(GC * (x + 0.044715 * (x * x * x))))


def _phi(x):
    return jnp.where(x > 0, x + 1.0, jnp.exp(x))


def _dot(a, b):
    return jnp.dot(a, b, preferred_element_type=F32)


def _dot_nt(a, b):
    return lax.dot_general(a, b, NT, preferred_element_type=F32)


def _head_mask(x, j):
    lane = lax.broadcasted_iota(jnp.int32, (1, 128), 1)
    m = jnp.where((lane >= 32 * j) & (lane < 32 * j + 32), -1, 0).astype(jnp.int32)
    return pltpu.bitcast(pltpu.bitcast(x, jnp.int32) & m, BF)


def _kernel(beta_ref, x_hbm, wq_hbm, wk_hbm, wv_hbm, wo_hbm, w1_hbm, w2_hbm, w3_hbm, w4_hbm,
            out_hbm,
            wq, wk, wv, wo, w1, w2, w3, w4,
            xf, xn_s, h_s, xio, qs, pq, ks, pk, vt, o_s, mst, gtab, sem, osem):
    def cp(src, dst, i):
        return pltpu.make_async_copy(src, dst, sem.at[i])
    c_x = cp(x_hbm.at[0], xio, 0)
    c_w = [cp(wq_hbm, wq, 1), cp(wk_hbm, wk, 2), cp(wv_hbm, wv, 3), cp(wo_hbm, wo, 4),
           cp(w1_hbm, w1, 5), cp(w2_hbm, w2, 6), cp(w3_hbm, w3, 7), cp(w4_hbm, w4, 8)]
    c_x.start()
    for c in c_w:
        c.start()

    b = beta_ref[...].astype(F32)
    hrow = lax.broadcasted_iota(jnp.int32, (H, H), 0)
    hcol = lax.broadcasted_iota(jnp.int32, (H, H), 1)
    bcol = jnp.sum(jnp.where(hrow == hcol, jnp.broadcast_to(b, (H, H)), 0.0), axis=1, keepdims=True)
    gtab[...] = jnp.broadcast_to(jax.nn.sigmoid(bcol), (H, 128))

    for g in range(NG):
        vt[g, 128:VR, :] = jnp.ones((VR - 128, L), BF)
    h_s[0:HPAD, :] = jnp.zeros((HPAD, D), F32)
    h_s[HPAD + S:HPAD + S + HPAD, :] = jnp.zeros((HPAD, D), F32)

    c_x.wait()

    def cvt(i, c):
        r = pl.multiple_of(i * L, L)
        xf[pl.ds(r, L), :] = xio[pl.ds(r, L), :].astype(F32)
        return c
    lax.fori_loop(0, NSEG, cvt, 0)

    row = lax.broadcasted_iota(jnp.int32, (128, 128), 0)
    col = lax.broadcasted_iota(jnp.int32, (128, 128), 1)

    def attention_groups(g0, ngroups):
        steps = [(gg, i, t) for gg in range(ngroups) for i in (3, 2, 1, 0) for t in range(i + 1)]
        ctx, wcache, state, mem = {}, {}, {}, {}

        def getg(gg):
            if gg not in ctx:
                g = g0 + gg
                c0 = pl.multiple_of(g * 128, 128)
                ctx[gg] = (g, c0, qs[:, pl.ds(c0, 128)], ks[:, pl.ds(c0, 128)], vt[g])
            return ctx[gg]

        def mem_read(gg):
            g, c0, _, _, vtg = getg(gg)
            nd = _dot_nt(mst[g].astype(BF), pq[:, pl.ds(c0, 128)])
            gates = [gtab[pl.ds(4 * g + j, 1), :] for j in range(4)]
            mem[gg] = (nd, gates)
            upd = _dot(vtg, pk[:, pl.ds(c0, 128)])
            r = lax.broadcasted_iota(jnp.int32, (VR, 128), 0)
            c = lax.broadcasted_iota(jnp.int32, (VR, 128), 1)
            keep = jnp.where(r < 128, r // 32, r - 128) == c // 32
            mst[g] = mst[g] + jnp.where(keep, upd, 0.0)

        def qk(st):
            gg, i, t = st
            _, _, qg, kg, _ = getg(gg)
            if (gg, i) not in wcache:
                qi = qg[128 * i:128 * (i + 1)]
                wcache[(gg, i)] = jnp.concatenate([_head_mask(qi, j) for j in range(4)], axis=0)
            return _dot_nt(kg[128 * t:128 * (t + 1)], wcache[(gg, i)])

        def pv(st, St):
            gg, i, t = st
            g, c0, _, _, vtg = getg(gg)
            accs, ls = state.setdefault((gg, i), ([None] * 4, [None] * 4))
            for j in range(4):
                P = jnp.exp2(St[:, 128 * j:128 * (j + 1)])
                if t == i:
                    P = jnp.where(row <= col, P, 0.0)
                ps = jnp.sum(P.reshape(16, 8, 128), axis=0)
                ls[j] = ps if ls[j] is None else ls[j] + ps
                O = _dot(vtg[32 * j:32 * j + 32, 128 * t:128 * (t + 1)], P.astype(BF))
                accs[j] = O if accs[j] is None else accs[j] + O
            if t == i:
                nd, gates = mem[gg]
                rows = []
                for j in range(4):
                    l = jnp.sum(ls[j], axis=0, keepdims=True)
                    gj = gates[j]
                    den = nd[128 + j:129 + j, 128 * i:128 * (i + 1)] + 1e-6
                    num = nd[32 * j:32 * j + 32, 128 * i:128 * (i + 1)]
                    rows.append(accs[j] * ((1.0 - gj) / l) + num * (gj / den))
                o_s[128 * i:128 * (i + 1), pl.ds(c0, 128)] = jnp.concatenate(rows, axis=0).T.astype(BF)

        LA = 2
        pend = []
        seen = set()
        for st in steps:
            if st[0] not in seen:
                seen.add(st[0])
                mem_read(st[0])
            pend.append((st, qk(st)))
            if len(pend) > LA:
                pv(*pend.pop(0))
        while pend:
            pv(*pend.pop(0))

    GPI = 4

    def layer(ell, carry):
        mst[...] = jnp.zeros((NG, VR, 128), F32)

        @pl.when(ell == 0)
        def _():
            for c in c_w[:3]:
                c.wait()

        def seg(s, c):
            r0 = pl.multiple_of(s * L, L)
            xnb = _ln(xf[pl.ds(r0, L), :]).astype(BF)
            q = _dot(xnb, wq[...])
            qs[...] = (q * QSCALE).astype(BF)
            pq[...] = _phi(q).astype(BF)
            k = _dot(xnb, wk[...])
            ks[...] = k.astype(BF)
            pk[...] = _phi(k).astype(BF)
            v = _dot(xnb, wv[...])
            for g in range(NG):
                vt[g, 0:128, :] = v[:, 128 * g:128 * (g + 1)].T.astype(BF)

            def att(it, c2):
                attention_groups(it * GPI, GPI)
                return c2
            lax.fori_loop(0, NG // GPI, att, 0)

            @pl.when(jnp.logical_and(ell == 0, s == 0))
            def _():
                for cw in c_w[3:5]:
                    cw.wait()

            for hb in range(2):
                rr = pl.multiple_of(r0 + hb * 256, 256)
                x = xf[pl.ds(rr, 256), :] + _dot(o_s[hb * 256:(hb + 1) * 256, :], wo[...])
                xf[pl.ds(rr, 256), :] = x
                xn = _ln(x)
                xn_s[pl.ds(rr, 256), :] = xn
                hh = _gelu(_dot(_ln(xn).astype(BF), w1[...]))
                h_s[pl.ds(pl.multiple_of(rr + HPAD, 8), 256), :] = hh
            return c
        lax.fori_loop(0, NSEG, seg, 0)

        @pl.when(ell == 0)
        def _():
            for cw in c_w[5:]:
                cw.wait()

        def blk(s, c):
            r0 = pl.multiple_of(s * L, L)
            for hb in range(2):
                rr = pl.multiple_of(r0 + hb * 256, 256)
                c4 = D // 4
                parts = []
                for ci, sh in enumerate((-1, 1, -2, 2)):
                    w0 = rr if sh < 0 else rr + HPAD
                    win = h_s[pl.ds(pl.multiple_of(w0, 8), 256 + HPAD), ci * c4:(ci + 1) * c4]
                    o0 = HPAD + sh if sh < 0 else sh
                    parts.append(win[o0:o0 + 256].astype(BF))
                hs = _dot(jnp.concatenate(parts, axis=1), w2[...])
                x1 = xn_s[pl.ds(rr, 256), :] + hs
                x1n = _ln(x1).astype(BF)
                acc = xf[pl.ds(rr, 256), :] + x1
                FC = 512
                for f in range(F // FC):
                    hh = _gelu(_dot(x1n, w3[:, f * FC:(f + 1) * FC])).astype(BF)
                    acc = acc + _dot(hh, w4[f * FC:(f + 1) * FC, :])
                xf[pl.ds(rr, 256), :] = acc
                xio[pl.ds(rr, 256), :] = acc.astype(BF)

            @pl.when(ell == 1)
            def _():
                pltpu.make_async_copy(xio.at[pl.ds(r0, L)], out_hbm.at[0, pl.ds(r0, L)], osem.at[s]).start()
            return c
        lax.fori_loop(0, NSEG, blk, 0)
        return carry

    lax.fori_loop(0, 2, layer, 0)
    for s in range(NSEG):
        pltpu.make_async_copy(xio.at[pl.ds(s * L, L)], out_hbm.at[0, pl.ds(s * L, L)], osem.at[s]).wait()


@jax.jit
def pallas_interleave_layers__memory_aug_infini_attn__mixer_s_mlp__prompt_kernel(
    A_x, A_wq, A_wk, A_wv, A_wo, A_beta, B_x, B_w1, B_w2, B_w3, B_w4,
):
    del B_x
    any_spec = pl.BlockSpec(memory_space=pl.ANY)
    vm = pltpu.VMEM
    scratch = [
        vm((D, D), BF), vm((D, D), BF), vm((D, D), BF), vm((D, D), BF),
        vm((D, D), BF), vm((D, D), BF), vm((D, F), BF), vm((F, D), BF),
        vm((S, D), F32), vm((S, D), F32), vm((S + 2 * HPAD, D), F32),
        vm((S, D), BF),
        vm((L, D), BF), vm((L, D), BF), vm((L, D), BF), vm((L, D), BF),
        vm((NG, VR, L), BF), vm((L, D), BF),
        vm((NG, VR, 128), F32), vm((H, 128), F32),
        pltpu.SemaphoreType.DMA((9,)), pltpu.SemaphoreType.DMA((NSEG,)),
    ]
    return pl.pallas_call(
        _kernel,
        out_shape=jax.ShapeDtypeStruct((1, S, D), BF),
        in_specs=[pl.BlockSpec(memory_space=pltpu.VMEM)] + [any_spec] * 9,
        out_specs=any_spec,
        scratch_shapes=scratch,
        compiler_params=pltpu.CompilerParams(vmem_limit_bytes=110 * 2 ** 20),
        name="fused_infini_mixer",
    )(A_beta.reshape(1, H), A_x, A_wq, A_wk, A_wv, A_wo, B_w1, B_w2, B_w3, B_w4)
```

```python
import functools

import numpy as np
import jax
import jax.numpy as jnp
from jax import lax
import jax.experimental.pallas as pl
import jax.experimental.pallas.tpu as pltpu

S, D, H, DH, NSEG, L, F = 2048, 1024, 32, 32, 4, 512, 3584
NG = D // 128
BF, F32 = jnp.bfloat16, jnp.float32
NT = (((1,), (1,)), ((), ()))
EPS = 1e-5
LOG2E = float(np.log2(np.e))
QSCALE = float(DH ** -0.5) * LOG2E
GC = float(np.sqrt(2.0 / np.pi))
HPAD = 8
L_LO, L_HI = 2.0 ** -40, 2.0 ** 40
MASKV = -1e9 * LOG2E
VR = 144


def _ln(x):
    m = jnp.mean(x, axis=-1, keepdims=True)
    xc = x - m
    v = jnp.mean(xc * xc, axis=-1, keepdims=True)
    return xc * lax.rsqrt(v + EPS)


def _gelu(x):
    return 0.5 * x * (1.0 + jnp.tanh(GC * (x + 0.044715 * (x * x * x))))


def _phi(x):
    return jnp.where(x > 0, x + 1.0, jnp.exp(x))


def _dot(a, b):
    return jnp.dot(a, b, preferred_element_type=F32)


def _dot_nt(a, b):
    return lax.dot_general(a, b, NT, preferred_element_type=F32)


def _head_mask(x, j):
    lane = lax.broadcasted_iota(jnp.int32, (1, 128), 1)
    m = jnp.where((lane >= 32 * j) & (lane < 32 * j + 32), -1, 0).astype(jnp.int32)
    return pltpu.bitcast(pltpu.bitcast(x, jnp.int32) & m, BF)


def _kernel(beta_ref, x_hbm, wq_hbm, wk_hbm, wv_hbm, wo_hbm, w1_hbm, w2_hbm, w3_hbm, w4_hbm,
            out_hbm,
            wq, wk, wv, wo, w1, w2, w3, w4,
            xf, xn_s, h_s, xio, qs, pq, ks, pk, vt, o_s, mst, gtab, sem, osem):
    def cp(src, dst, i):
        return pltpu.make_async_copy(src, dst, sem.at[i])
    c_x = cp(x_hbm.at[0], xio, 0)
    c_w = [cp(wq_hbm, wq, 1), cp(wk_hbm, wk, 2), cp(wv_hbm, wv, 3), cp(wo_hbm, wo, 4),
           cp(w1_hbm, w1, 5), cp(w2_hbm, w2, 6), cp(w3_hbm, w3, 7), cp(w4_hbm, w4, 8)]
    c_x.start()
    for c in c_w:
        c.start()

    b = beta_ref[...].astype(F32)
    hrow = lax.broadcasted_iota(jnp.int32, (H, H), 0)
    hcol = lax.broadcasted_iota(jnp.int32, (H, H), 1)
    bcol = jnp.sum(jnp.where(hrow == hcol, jnp.broadcast_to(b, (H, H)), 0.0), axis=1, keepdims=True)
    gtab[...] = jnp.broadcast_to(jax.nn.sigmoid(bcol), (H, 128))

    for g in range(NG):
        vt[g, 128:VR, :] = jnp.ones((VR - 128, L), BF)
    h_s[0:HPAD, :] = jnp.zeros((HPAD, D), F32)
    h_s[HPAD + S:HPAD + S + HPAD, :] = jnp.zeros((HPAD, D), F32)

    c_x.wait()

    def cvt(i, c):
        r = pl.multiple_of(i * L, L)
        xf[pl.ds(r, L), :] = xio[pl.ds(r, L), :].astype(F32)
        return c
    lax.fori_loop(0, NSEG, cvt, 0)

    row = lax.broadcasted_iota(jnp.int32, (128, 128), 0)
    col = lax.broadcasted_iota(jnp.int32, (128, 128), 1)

    def attention_groups(g0, ngroups, par, bad):
        flag = [bad]
        steps = [(gg, i, t) for gg in range(ngroups) for i in (3, 2, 1, 0) for t in range(i + 1)]
        ctx, wcache, state, mem = {}, {}, {}, {}

        def getg(gg):
            if gg not in ctx:
                g = g0 + gg
                c0 = pl.multiple_of(g * 128, 128)
                ctx[gg] = (g, c0, qs[:, pl.ds(c0, 128)], ks[:, pl.ds(c0, 128)], vt[g])
            return ctx[gg]

        def mem_read(gg):
            g, c0, _, _, vtg = getg(gg)
            m_old = mst[par, g]
            nd = _dot_nt(m_old.astype(BF), pq[:, pl.ds(c0, 128)])
            gates = [gtab[pl.ds(4 * g + j, 1), :] for j in range(4)]
            mem[gg] = (nd, gates)
            upd = _dot(vtg, pk[:, pl.ds(c0, 128)])
            r = lax.broadcasted_iota(jnp.int32, (VR, 128), 0)
            c = lax.broadcasted_iota(jnp.int32, (VR, 128), 1)
            keep = jnp.where(r < 128, r // 32, r - 128) == c // 32
            mst[1 - par, g] = m_old + jnp.where(keep, upd, 0.0)

        def qk(st):
            gg, i, t = st
            _, _, qg, kg, _ = getg(gg)
            if (gg, i) not in wcache:
                qi = qg[128 * i:128 * (i + 1)]
                wcache[(gg, i)] = jnp.concatenate([_head_mask(qi, j) for j in range(4)], axis=0)
            return _dot_nt(kg[128 * t:128 * (t + 1)], wcache[(gg, i)])

        def pv(st, St):
            gg, i, t = st
            g, c0, _, _, vtg = getg(gg)
            accs, ls = state.setdefault((gg, i), ([None] * 4, [None] * 4))
            for j in range(4):
                P = jnp.exp2(St[:, 128 * j:128 * (j + 1)])
                if t == i:
                    P = jnp.where(row <= col, P, 0.0)
                ps = jnp.sum(P.reshape(16, 8, 128), axis=0)
                ls[j] = ps if ls[j] is None else ls[j] + ps
                O = _dot(vtg[32 * j:32 * j + 32, 128 * t:128 * (t + 1)], P.astype(BF))
                accs[j] = O if accs[j] is None else accs[j] + O
            if t == i:
                nd, gates = mem[gg]
                rows = []
                for j in range(4):
                    l = jnp.sum(ls[j], axis=0, keepdims=True)
                    flag[0] = jnp.where((l >= L_LO) & (l <= L_HI), flag[0], 1.0)
                    gj = gates[j]
                    den = nd[128 + j:129 + j, 128 * i:128 * (i + 1)] + 1e-6
                    num = nd[32 * j:32 * j + 32, 128 * i:128 * (i + 1)]
                    rows.append(accs[j] * ((1.0 - gj) / l) + num * (gj / den))
                o_s[128 * i:128 * (i + 1), pl.ds(c0, 128)] = jnp.concatenate(rows, axis=0).T.astype(BF)

        LA = 2
        pend = []
        seen = set()
        for st in steps:
            if st[0] not in seen:
                seen.add(st[0])
                mem_read(st[0])
            pend.append((st, qk(st)))
            if len(pend) > LA:
                pv(*pend.pop(0))
        while pend:
            pv(*pend.pop(0))
        return flag[0]

    def attention_safe(par):
        def body(n, c):
            g, i = n // 4, n % 4
            c0 = pl.multiple_of(g * 128, 128)
            q0 = pl.multiple_of(i * 128, 128)
            qi = qs[pl.ds(q0, 128), pl.ds(c0, 128)]
            W = jnp.concatenate([_head_mask(qi, j) for j in range(4)], axis=0)
            kr = lax.broadcasted_iota(jnp.int32, (128, 512), 0)
            qc = lax.broadcasted_iota(jnp.int32, (128, 512), 1) & 127

            def logits(t):
                k0 = pl.multiple_of(t * 128, 128)
                St = _dot_nt(ks[pl.ds(k0, 128), pl.ds(c0, 128)], W)
                return St + jnp.where(kr + k0 > qc + q0, MASKV, 0.0), k0

            def pass1(t, m):
                return jnp.maximum(m, jnp.max(logits(t)[0], axis=0, keepdims=True))
            m = lax.fori_loop(0, i + 1, pass1, jnp.full((1, 512), -jnp.inf, F32))

            def pass2(t, carry):
                acc, l = carry
                St, k0 = logits(t)
                P = jnp.exp2(St - m)
                outs = [_dot(vt[g, 32 * j:32 * j + 32, pl.ds(k0, 128)],
                             P[:, 128 * j:128 * (j + 1)].astype(BF)) for j in range(4)]
                return acc + jnp.concatenate(outs, axis=0), l + jnp.sum(P, axis=0, keepdims=True)
            acc, l = lax.fori_loop(0, i + 1, pass2,
                                   (jnp.zeros((128, 128), F32), jnp.zeros((1, 512), F32)))

            nd = _dot_nt(mst[par, g].astype(BF), pq[pl.ds(q0, 128), pl.ds(c0, 128)])
            rows = []
            for j in range(4):
                gj = gtab[pl.ds(4 * g + j, 1), :]
                den = nd[128 + j:129 + j, :] + 1e-6
                rows.append(acc[32 * j:32 * j + 32] * ((1.0 - gj) / l[:, 128 * j:128 * (j + 1)])
                            + nd[32 * j:32 * j + 32] * (gj / den))
            o_s[pl.ds(q0, 128), pl.ds(c0, 128)] = jnp.concatenate(rows, axis=0).T.astype(BF)
            return c
        lax.fori_loop(0, NG * 4, body, 0)

    GPI = 4
    RB, CH = 256, 128
    NCH = RB // CH

    def layer(ell, carry):
        mst[0] = jnp.zeros((NG, VR, 128), F32)

        @pl.when(ell == 0)
        def _():
            for c in c_w[:3]:
                c.wait()

        def seg(s, c):
            r0 = pl.multiple_of(s * L, L)

            def qkv(u, c1):
                offs = [pl.multiple_of(u * RB + ch * CH, CH) for ch in range(NCH)]
                xnb = [_ln(xf[pl.ds(r0 + o, CH), :]).astype(BF) for o in offs]
                for o, xb in zip(offs, xnb):
                    q = _dot(xb, wq[...])
                    qs[pl.ds(o, CH), :] = (q * QSCALE).astype(BF)
                    pq[pl.ds(o, CH), :] = _phi(q).astype(BF)
                for o, xb in zip(offs, xnb):
                    k = _dot(xb, wk[...])
                    ks[pl.ds(o, CH), :] = k.astype(BF)
                    pk[pl.ds(o, CH), :] = _phi(k).astype(BF)
                for o, xb in zip(offs, xnb):
                    v = _dot(xb, wv[...])
                    for g in range(NG):
                        vt[g, 0:128, pl.ds(o, CH)] = v[:, 128 * g:128 * (g + 1)].T.astype(BF)
                return c1
            lax.fori_loop(0, L // RB, qkv, 0)

            par = s % 2
            bad = lax.fori_loop(0, NG // GPI,
                                lambda it, b: attention_groups(it * GPI, GPI, par, b),
                                jnp.zeros((1, 128), F32))

            @pl.when(jnp.max(bad) > 0.0)
            def _():
                attention_safe(par)

            @pl.when(jnp.logical_and(ell == 0, s == 0))
            def _():
                for cw in c_w[3:5]:
                    cw.wait()

            def proj(u, c3):
                offs = [pl.multiple_of(u * RB + ch * CH, CH) for ch in range(NCH)]
                xs = []
                for o in offs:
                    x = xf[pl.ds(r0 + o, CH), :] + _dot(o_s[pl.ds(o, CH), :], wo[...])
                    xf[pl.ds(r0 + o, CH), :] = x
                    xs.append(x)
                for o, x in zip(offs, xs):
                    xn = _ln(x)
                    xn_s[pl.ds(r0 + o, CH), :] = xn
                    h_s[pl.ds(pl.multiple_of(r0 + o + HPAD, 8), CH), :] = _gelu(_dot(_ln(xn).astype(BF), w1[...]))
                return c3
            lax.fori_loop(0, L // RB, proj, 0)
            return c
        lax.fori_loop(0, NSEG, seg, 0)

        @pl.when(ell == 0)
        def _():
            for cw in c_w[5:]:
                cw.wait()

        def blk(s, c):
            r0 = pl.multiple_of(s * RB, RB)
            offs = [pl.multiple_of(r0 + ch * CH, CH) for ch in range(NCH)]
            c4 = D // 4
            hss = []
            for rr in offs:
                parts = []
                for ci, sh in enumerate((-1, 1, -2, 2)):
                    w0 = rr if sh < 0 else rr + HPAD
                    win = h_s[pl.ds(pl.multiple_of(w0, 8), CH + HPAD), ci * c4:(ci + 1) * c4]
                    o0 = HPAD + sh if sh < 0 else sh
                    parts.append(win[o0:o0 + CH].astype(BF))
                hss.append(_dot(jnp.concatenate(parts, axis=1), w2[...]))
            FC = 512
            for rr, hs in zip(offs, hss):
                x1 = xn_s[pl.ds(rr, CH), :] + hs
                x1n = _ln(x1).astype(BF)
                acc = xf[pl.ds(rr, CH), :] + x1
                for f in range(F // FC):
                    hh = _gelu(_dot(x1n, w3[:, f * FC:(f + 1) * FC])).astype(BF)
                    acc = acc + _dot(hh, w4[f * FC:(f + 1) * FC, :])
                xf[pl.ds(rr, CH), :] = acc
                xio[pl.ds(rr, CH), :] = acc.astype(BF)

            @pl.when(ell == 1)
            def _():
                pltpu.make_async_copy(xio.at[pl.ds(r0, RB)], out_hbm.at[0, pl.ds(r0, RB)], osem.at[s]).start()
            return c
        lax.fori_loop(0, S // RB, blk, 0)
        return carry

    lax.fori_loop(0, 2, layer, 0)
    for s in range(S // RB):
        pltpu.make_async_copy(xio.at[pl.ds(s * RB, RB)], out_hbm.at[0, pl.ds(s * RB, RB)], osem.at[s]).wait()


@jax.jit
def pallas_interleave_layers__memory_aug_infini_attn__mixer_s_mlp__prompt_kernel(
    A_x, A_wq, A_wk, A_wv, A_wo, A_beta, B_x, B_w1, B_w2, B_w3, B_w4,
):
    del B_x
    any_spec = pl.BlockSpec(memory_space=pl.ANY)
    vm = pltpu.VMEM
    scratch = [
        vm((D, D), BF), vm((D, D), BF), vm((D, D), BF), vm((D, D), BF),
        vm((D, D), BF), vm((D, D), BF), vm((D, F), BF), vm((F, D), BF),
        vm((S, D), F32), vm((S, D), F32), vm((S + 2 * HPAD, D), F32),
        vm((S, D), BF),
        vm((L, D), BF), vm((L, D), BF), vm((L, D), BF), vm((L, D), BF),
        vm((NG, VR, L), BF), vm((L, D), BF),
        vm((2, NG, VR, 128), F32), vm((H, 128), F32),
        pltpu.SemaphoreType.DMA((9,)), pltpu.SemaphoreType.DMA((8,)),
    ]
    return pl.pallas_call(
        _kernel,
        out_shape=jax.ShapeDtypeStruct((1, S, D), BF),
        in_specs=[pl.BlockSpec(memory_space=pltpu.VMEM)] + [any_spec] * 9,
        out_specs=any_spec,
        scratch_shapes=scratch,
        compiler_params=pltpu.CompilerParams(vmem_limit_bytes=110 * 2 ** 20),
        name="fused_infini_mixer",
    )(A_beta.reshape(1, H), A_x, A_wq, A_wk, A_wv, A_wo, B_w1, B_w2, B_w3, B_w4)
```

```python
import functools

import numpy as np
import jax
import jax.numpy as jnp
from jax import lax
import jax.experimental.pallas as pl
import jax.experimental.pallas.tpu as pltpu

S, D, H, DH, NSEG, L, F = 2048, 1024, 32, 32, 4, 512, 3584
NG = D // 128
BF, F32 = jnp.bfloat16, jnp.float32
NT = (((1,), (1,)), ((), ()))
EPS = 1e-5
LOG2E = float(np.log2(np.e))
QSCALE = float(DH ** -0.5) * LOG2E
GC = float(np.sqrt(2.0 / np.pi))
HPAD = 8
L_LO, L_HI = 2.0 ** -40, 2.0 ** 40
MASKV = -1e9 * LOG2E
GPI = 4
RB, CH = 256, 128
NCH = RB // CH
VR = 144


def _ln(x):
    m = jnp.mean(x, axis=-1, keepdims=True)
    xc = x - m
    v = jnp.mean(xc * xc, axis=-1, keepdims=True)
    return xc * lax.rsqrt(v + EPS)


def _gelu(x):
    return 0.5 * x * (1.0 + jnp.tanh(GC * (x + 0.044715 * (x * x * x))))


def _phi(x):
    return jnp.where(x > 0, x + 1.0, jnp.exp(x))


def _dot(a, b):
    return jnp.dot(a, b, preferred_element_type=F32)


def _dot_nt(a, b):
    return lax.dot_general(a, b, NT, preferred_element_type=F32)


def _head_mask(x, j):
    lane = lax.broadcasted_iota(jnp.int32, (1, 128), 1)
    m = jnp.where((lane >= 32 * j) & (lane < 32 * j + 32), -1, 0).astype(jnp.int32)
    return pltpu.bitcast(pltpu.bitcast(x, jnp.int32) & m, BF)


def _kernel(beta_ref, x_hbm, wq_hbm, wk_hbm, wv_hbm, wo_hbm, w1_hbm, w2_hbm, w3_hbm, w4_hbm,
            out_hbm,
            wq, wk, wv, wo, w1, w2, w3, w4,
            xf, xn_s, h_s, xio, xnb, qs, pq, ks, pk, vt, o_s, mst, gtab, sem, osem):
    def cp(src, dst, i):
        return pltpu.make_async_copy(src, dst, sem.at[i])
    NB = S // RB

    def c_xb(i):
        r = pl.multiple_of(i * RB, RB)
        return cp(x_hbm.at[0, pl.ds(r, RB)], xio.at[pl.ds(r, RB)], 9 + i)
    c_w = [cp(wv_hbm, wv, 1), cp(wq_hbm, wq, 2), cp(wk_hbm, wk, 3), cp(wo_hbm, wo, 4),
           cp(w1_hbm, w1, 5), cp(w2_hbm, w2, 6), cp(w3_hbm, w3, 7), cp(w4_hbm, w4, 8)]
    for c in [c_xb(0), c_xb(1), c_xb(2)] + c_w[:3]:
        c.start()

    b = beta_ref[...].astype(F32)
    hrow = lax.broadcasted_iota(jnp.int32, (H, H), 0)
    hcol = lax.broadcasted_iota(jnp.int32, (H, H), 1)
    bcol = jnp.sum(jnp.where(hrow == hcol, jnp.broadcast_to(b, (H, H)), 0.0), axis=1, keepdims=True)
    gtab[...] = jnp.broadcast_to(jax.nn.sigmoid(bcol), (H, 128))

    for g in range(NG):
        vt[g, 128:VR, :] = jnp.ones((VR - 128, L), BF)
    h_s[0:HPAD, :] = jnp.zeros((HPAD, D), F32)
    h_s[HPAD + S:HPAD + S + HPAD, :] = jnp.zeros((HPAD, D), F32)

    def cvt(i, c):
        c_xb(i).wait()
        r = pl.multiple_of(i * RB, RB)
        xf[pl.ds(r, RB), :] = xio[pl.ds(r, RB), :].astype(F32)
        return c
    lax.fori_loop(0, 2, cvt, 0)

    row = lax.broadcasted_iota(jnp.int32, (128, 128), 0)
    col = lax.broadcasted_iota(jnp.int32, (128, 128), 1)

    def attention_groups(g0, ngroups, par, bad):
        flag = [bad]
        steps = [(gg, i, t) for gg in range(ngroups) for i in (3, 2, 1, 0) for t in range(i + 1)]
        ctx, wcache, state, mem = {}, {}, {}, {}

        def getg(gg):
            if gg not in ctx:
                g = g0 + gg
                c0 = pl.multiple_of(g * 128, 128)
                ctx[gg] = (g, c0, qs[:, pl.ds(c0, 128)], ks[:, pl.ds(c0, 128)], vt[g])
            return ctx[gg]

        def mem_read(gg):
            g, c0, _, _, vtg = getg(gg)
            m_old = mst[par, g]
            nd = _dot_nt(m_old.astype(BF), pq[:, pl.ds(c0, 128)])
            gates = [gtab[pl.ds(4 * g + j, 1), :] for j in range(4)]
            mem[gg] = (nd, gates)
            upd = _dot(vtg, pk[:, pl.ds(c0, 128)])
            r = lax.broadcasted_iota(jnp.int32, (VR, 128), 0)
            c = lax.broadcasted_iota(jnp.int32, (VR, 128), 1)
            keep = jnp.where(r < 128, r // 32, r - 128) == c // 32
            mst[1 - par, g] = m_old + jnp.where(keep, upd, 0.0)

        def qk(st):
            gg, i, t = st
            _, _, qg, kg, _ = getg(gg)
            if (gg, i) not in wcache:
                qi = qg[128 * i:128 * (i + 1)]
                wcache[(gg, i)] = jnp.concatenate([_head_mask(qi, j) for j in range(4)], axis=0)
            return _dot_nt(kg[128 * t:128 * (t + 1)], wcache[(gg, i)])

        def pv(st, St):
            gg, i, t = st
            g, c0, _, _, vtg = getg(gg)
            accs, ls = state.setdefault((gg, i), ([None] * 4, [None] * 4))
            for j in range(4):
                P = jnp.exp2(St[:, 128 * j:128 * (j + 1)])
                if t == i:
                    P = jnp.where(row <= col, P, 0.0)
                ps = jnp.sum(P.reshape(16, 8, 128), axis=0)
                ls[j] = ps if ls[j] is None else ls[j] + ps
                O = _dot(vtg[32 * j:32 * j + 32, 128 * t:128 * (t + 1)], P.astype(BF))
                accs[j] = O if accs[j] is None else accs[j] + O
            if t == i:
                nd, gates = mem[gg]
                rows = []
                for j in range(4):
                    l = jnp.sum(ls[j], axis=0, keepdims=True)
                    flag[0] = jnp.where((l >= L_LO) & (l <= L_HI), flag[0], 1.0)
                    gj = gates[j]
                    den = nd[128 + j:129 + j, 128 * i:128 * (i + 1)] + 1e-6
                    num = nd[32 * j:32 * j + 32, 128 * i:128 * (i + 1)]
                    rows.append(accs[j] * ((1.0 - gj) / l) + num * (gj / den))
                o_s[128 * i:128 * (i + 1), pl.ds(c0, 128)] = jnp.concatenate(rows, axis=0).T.astype(BF)

        LA = 2
        pend = []
        seen = set()
        for st in steps:
            if st[0] not in seen:
                seen.add(st[0])
                mem_read(st[0])
            pend.append((st, qk(st)))
            if len(pend) > LA:
                pv(*pend.pop(0))
        while pend:
            pv(*pend.pop(0))
        return flag[0]

    def attention_safe(par):
        def body(n, c):
            g, i = n // 4, n % 4
            c0 = pl.multiple_of(g * 128, 128)
            q0 = pl.multiple_of(i * 128, 128)
            qi = qs[pl.ds(q0, 128), pl.ds(c0, 128)]
            W = jnp.concatenate([_head_mask(qi, j) for j in range(4)], axis=0)
            kr = lax.broadcasted_iota(jnp.int32, (128, 512), 0)
            qc = lax.broadcasted_iota(jnp.int32, (128, 512), 1) & 127

            def logits(t):
                k0 = pl.multiple_of(t * 128, 128)
                St = _dot_nt(ks[pl.ds(k0, 128), pl.ds(c0, 128)], W)
                return St + jnp.where(kr + k0 > qc + q0, MASKV, 0.0), k0

            def pass1(t, m):
                return jnp.maximum(m, jnp.max(logits(t)[0], axis=0, keepdims=True))
            m = lax.fori_loop(0, i + 1, pass1, jnp.full((1, 512), -jnp.inf, F32))

            def pass2(t, carry):
                acc, l = carry
                St, k0 = logits(t)
                P = jnp.exp2(St - m)
                outs = [_dot(vt[g, 32 * j:32 * j + 32, pl.ds(k0, 128)],
                             P[:, 128 * j:128 * (j + 1)].astype(BF)) for j in range(4)]
                return acc + jnp.concatenate(outs, axis=0), l + jnp.sum(P, axis=0, keepdims=True)
            acc, l = lax.fori_loop(0, i + 1, pass2,
                                   (jnp.zeros((128, 128), F32), jnp.zeros((1, 512), F32)))

            nd = _dot_nt(mst[par, g].astype(BF), pq[pl.ds(q0, 128), pl.ds(c0, 128)])
            rows = []
            for j in range(4):
                gj = gtab[pl.ds(4 * g + j, 1), :]
                den = nd[128 + j:129 + j, :] + 1e-6
                rows.append(acc[32 * j:32 * j + 32] * ((1.0 - gj) / l[:, 128 * j:128 * (j + 1)])
                            + nd[32 * j:32 * j + 32] * (gj / den))
            o_s[pl.ds(q0, 128), pl.ds(c0, 128)] = jnp.concatenate(rows, axis=0).T.astype(BF)
            return c
        lax.fori_loop(0, NG * 4, body, 0)

    def layer(ell, carry):
        mst[0] = jnp.zeros((NG, VR, 128), F32)
        xnb[0:RB, :] = _ln(xf[0:RB, :]).astype(BF)

        @pl.when(ell == 0)
        def _():
            cvt(2, 0)
            for c in c_w[:3]:
                c.wait()
            for i in range(3, NB):
                c_xb(i).start()
            for c in c_w[3:5]:
                c.start()

        def seg(s, c):
            r0 = pl.multiple_of(s * L, L)

            def qkv(u, c1):
                offs = [pl.multiple_of(u * RB + ch * CH, CH) for ch in range(NCH)]
                xbs = [xnb[pl.ds(r0 + o, CH), :] for o in offs]
                for o, xb in zip(offs, xbs):
                    v = _dot(xb, wv[...])
                    for g in range(NG):
                        vt[g, 0:128, pl.ds(o, CH)] = v[:, 128 * g:128 * (g + 1)].T.astype(BF)
                rn = pl.multiple_of(jnp.minimum(r0 + (u + 1) * RB, S - RB), RB)
                xnb[pl.ds(rn, RB), :] = _ln(xf[pl.ds(rn, RB), :]).astype(BF)
                for o, xb in zip(offs, xbs):
                    q = _dot(xb, wq[...])
                    qs[pl.ds(o, CH), :] = (q * QSCALE).astype(BF)
                    pq[pl.ds(o, CH), :] = _phi(q).astype(BF)
                for o in offs:
                    k = _dot(xnb[pl.ds(r0 + o, CH), :], wk[...])
                    ks[pl.ds(o, CH), :] = k.astype(BF)
                    pk[pl.ds(o, CH), :] = _phi(k).astype(BF)
                return c1

            lax.fori_loop(0, L // RB, qkv, 0)

            @pl.when((ell == 0) & (s < NSEG - 1))
            def _():
                nb = (s + 1) * (L // RB) + 1
                lax.fori_loop(nb, jnp.minimum(nb + L // RB, NB), cvt, 0)

            par = s % 2
            bad = lax.fori_loop(0, NG // GPI,
                                lambda it, b: attention_groups(it * GPI, GPI, par, b),
                                jnp.zeros((1, 128), F32))

            @pl.when(jnp.max(bad) > 0.0)
            def _():
                attention_safe(par)

            @pl.when(jnp.logical_and(ell == 0, s == 0))
            def _():
                for cw in c_w[3:5]:
                    cw.wait()
                for cw in c_w[5:]:
                    cw.start()

            def proj(u, c3):
                offs = [pl.multiple_of(u * RB + ch * CH, CH) for ch in range(NCH)]
                xs = []
                for o in offs:
                    x = xf[pl.ds(r0 + o, CH), :] + _dot(o_s[pl.ds(o, CH), :], wo[...])
                    xf[pl.ds(r0 + o, CH), :] = x
                    xs.append(x)
                for o, x in zip(offs, xs):
                    xn = _ln(x)
                    xn_s[pl.ds(r0 + o, CH), :] = xn
                    h_s[pl.ds(pl.multiple_of(r0 + o + HPAD, 8), CH), :] = _gelu(_dot(_ln(xn).astype(BF), w1[...]))
                return c3
            lax.fori_loop(0, L // RB, proj, 0)
            return c
        lax.fori_loop(0, NSEG, seg, 0)

        @pl.when(ell == 0)
        def _():
            for cw in c_w[5:]:
                cw.wait()

        def blk(s, c):
            r0 = pl.multiple_of(s * RB, RB)
            offs = [pl.multiple_of(r0 + ch * CH, CH) for ch in range(NCH)]
            c4 = D // 4
            hss = []
            for rr in offs:
                parts = []
                for ci, sh in enumerate((-1, 1, -2, 2)):
                    w0 = rr if sh < 0 else rr + HPAD
                    win = h_s[pl.ds(pl.multiple_of(w0, 8), CH + HPAD), ci * c4:(ci + 1) * c4]
                    o0 = HPAD + sh if sh < 0 else sh
                    parts.append(win[o0:o0 + CH].astype(BF))
                hss.append(_dot(jnp.concatenate(parts, axis=1), w2[...]))
            FC = 512
            for rr, hs in zip(offs, hss):
                x1 = xn_s[pl.ds(rr, CH), :] + hs
                x1n = _ln(x1).astype(BF)
                acc = xf[pl.ds(rr, CH), :] + x1
                for f in range(F // FC):
                    hh = _gelu(_dot(x1n, w3[:, f * FC:(f + 1) * FC])).astype(BF)
                    acc = acc + _dot(hh, w4[f * FC:(f + 1) * FC, :])
                xf[pl.ds(rr, CH), :] = acc
                xio[pl.ds(rr, CH), :] = acc.astype(BF)

            @pl.when(ell == 1)
            def _():
                pltpu.make_async_copy(xio.at[pl.ds(r0, RB)], out_hbm.at[0, pl.ds(r0, RB)], osem.at[s]).start()
            return c
        lax.fori_loop(0, S // RB, blk, 0)
        return carry

    lax.fori_loop(0, 2, layer, 0)
    for s in range(S // RB):
        pltpu.make_async_copy(xio.at[pl.ds(s * RB, RB)], out_hbm.at[0, pl.ds(s * RB, RB)], osem.at[s]).wait()


@jax.jit
def pallas_interleave_layers__memory_aug_infini_attn__mixer_s_mlp__prompt_kernel(
    A_x, A_wq, A_wk, A_wv, A_wo, A_beta, B_x, B_w1, B_w2, B_w3, B_w4,
):
    del B_x
    any_spec = pl.BlockSpec(memory_space=pl.ANY)
    vm = pltpu.VMEM
    scratch = [
        vm((D, D), BF), vm((D, D), BF), vm((D, D), BF), vm((D, D), BF),
        vm((D, D), BF), vm((D, D), BF), vm((D, F), BF), vm((F, D), BF),
        vm((S, D), F32), vm((S, D), F32), vm((S + 2 * HPAD, D), F32),
        vm((S, D), BF), vm((S, D), BF),
        vm((L, D), BF), vm((L, D), BF), vm((L, D), BF), vm((L, D), BF),
        vm((NG, VR, L), BF), vm((L, D), BF),
        vm((2, NG, VR, 128), F32), vm((H, 128), F32),
        pltpu.SemaphoreType.DMA((9 + S // RB,)), pltpu.SemaphoreType.DMA((8,)),
    ]
    return pl.pallas_call(
        _kernel,
        out_shape=jax.ShapeDtypeStruct((1, S, D), BF),
        in_specs=[pl.BlockSpec(memory_space=pltpu.VMEM)] + [any_spec] * 9,
        out_specs=any_spec,
        scratch_shapes=scratch,
        compiler_params=pltpu.CompilerParams(vmem_limit_bytes=110 * 2 ** 20),
        name="fused_infini_mixer",
    )(A_beta.reshape(1, H), A_x, A_wq, A_wk, A_wv, A_wo, B_w1, B_w2, B_w3, B_w4)
```

```python
import functools

import numpy as np
import jax
import jax.numpy as jnp
from jax import lax
import jax.experimental.pallas as pl
import jax.experimental.pallas.tpu as pltpu

S, D, H, DH, NSEG, L, F = 2048, 1024, 32, 32, 4, 512, 3584
NG = D // 128
BF, F32 = jnp.bfloat16, jnp.float32
NT = (((1,), (1,)), ((), ()))
EPS = 1e-5
LOG2E = float(np.log2(np.e))
QSCALE = float(DH ** -0.5) * LOG2E
GC = float(np.sqrt(2.0 / np.pi))
HPAD = 8
L_LO, L_HI = 2.0 ** -40, 2.0 ** 40
MASKV = -1e9 * LOG2E
GPI = 4
LA = 2
RB = 256
QCH, PCH, BCH = 128, 128, 128
FC = 896
VR = 144


def _ln(x):
    m = jnp.mean(x, axis=-1, keepdims=True)
    xc = x - m
    v = jnp.mean(xc * xc, axis=-1, keepdims=True)
    return xc * lax.rsqrt(v + EPS)


def _gelu(x):
    return 0.5 * x * (1.0 + jnp.tanh(GC * (x + 0.044715 * (x * x * x))))


def _phi(x):
    return jnp.where(x > 0, x + 1.0, jnp.exp(x))


def _dot(a, b):
    return jnp.dot(a, b, preferred_element_type=F32)


def _dot_nt(a, b):
    return lax.dot_general(a, b, NT, preferred_element_type=F32)


def _head_mask(x, j):
    lane = lax.broadcasted_iota(jnp.int32, (1, 128), 1)
    m = jnp.where((lane >= 32 * j) & (lane < 32 * j + 32), -1, 0).astype(jnp.int32)
    return pltpu.bitcast(pltpu.bitcast(x, jnp.int32) & m, BF)


def _kernel(beta_ref, x_hbm, wq_hbm, wk_hbm, wv_hbm, wo_hbm, w1_hbm, w2_hbm, w3_hbm, w4_hbm,
            out_hbm,
            wq, wk, wv, wo, w1, w2, w3, w4,
            xf, xn_s, h_s, xio, xnb, qs, pq, ks, pk, vt, o_s, mst, gtab, sem, osem):
    def cp(src, dst, i):
        return pltpu.make_async_copy(src, dst, sem.at[i])
    NB = S // RB

    def c_xb(i):
        r = pl.multiple_of(i * RB, RB)
        return cp(x_hbm.at[0, pl.ds(r, RB)], xio.at[pl.ds(r, RB)], 9 + i)
    c_w = [cp(wv_hbm, wv, 1), cp(wq_hbm, wq, 2), cp(wk_hbm, wk, 3), cp(wo_hbm, wo, 4),
           cp(w1_hbm, w1, 5), cp(w2_hbm, w2, 6), cp(w3_hbm, w3, 7), cp(w4_hbm, w4, 8)]
    for c in [c_xb(0), c_xb(1), c_xb(2)] + c_w[:3]:
        c.start()

    b = beta_ref[...].astype(F32)
    hrow = lax.broadcasted_iota(jnp.int32, (H, H), 0)
    hcol = lax.broadcasted_iota(jnp.int32, (H, H), 1)
    bcol = jnp.sum(jnp.where(hrow == hcol, jnp.broadcast_to(b, (H, H)), 0.0), axis=1, keepdims=True)
    gtab[...] = jnp.broadcast_to(jax.nn.sigmoid(bcol), (H, 128))

    for g in range(NG):
        vt[g, 128:VR, :] = jnp.ones((VR - 128, L), BF)
    h_s[0:HPAD, :] = jnp.zeros((HPAD, D), F32)
    h_s[HPAD + S:HPAD + S + HPAD, :] = jnp.zeros((HPAD, D), F32)

    def cvt(i, c):
        c_xb(i).wait()
        r = pl.multiple_of(i * RB, RB)
        xf[pl.ds(r, RB), :] = xio[pl.ds(r, RB), :].astype(F32)
        return c
    lax.fori_loop(0, 2, cvt, 0)

    row = lax.broadcasted_iota(jnp.int32, (128, 128), 0)
    col = lax.broadcasted_iota(jnp.int32, (128, 128), 1)

    def attention_groups(g0, ngroups, par, bad):
        flag = [bad]
        steps = [(gg, i, t) for gg in range(ngroups) for i in (3, 2, 1, 0) for t in range(i + 1)]
        ctx, wcache, state, mem = {}, {}, {}, {}

        def getg(gg):
            if gg not in ctx:
                g = g0 + gg
                c0 = pl.multiple_of(g * 128, 128)
                ctx[gg] = (g, c0, qs[:, pl.ds(c0, 128)], ks[:, pl.ds(c0, 128)], vt[g])
            return ctx[gg]

        def mem_read(gg):
            g, c0, _, _, vtg = getg(gg)
            nd = _dot_nt(mst[par, g].astype(BF), pq[:, pl.ds(c0, 128)])
            gates = [gtab[pl.ds(4 * g + j, 1), :] for j in range(4)]
            mem[gg] = (nd, gates)

        def mem_update(gg):
            g, c0, _, _, vtg = getg(gg)
            upd = _dot(vtg, pk[:, pl.ds(c0, 128)])
            r = lax.broadcasted_iota(jnp.int32, (VR, 128), 0)
            c = lax.broadcasted_iota(jnp.int32, (VR, 128), 1)
            keep = jnp.where(r < 128, r // 32, r - 128) == c // 32
            mst[1 - par, g] = mst[par, g] + jnp.where(keep, upd, 0.0)

        def qk(st):
            gg, i, t = st
            _, _, qg, kg, _ = getg(gg)
            if (gg, i) not in wcache:
                qi = qg[128 * i:128 * (i + 1)]
                wcache[(gg, i)] = jnp.concatenate([_head_mask(qi, j) for j in range(4)], axis=0)
            return _dot_nt(kg[128 * t:128 * (t + 1)], wcache[(gg, i)])

        def pv(st, St):
            gg, i, t = st
            g, c0, _, _, vtg = getg(gg)
            accs, ls = state.setdefault((gg, i), ([None] * 4, [None] * 4))
            for j in range(4):
                P = jnp.exp2(St[:, 128 * j:128 * (j + 1)])
                if t == i:
                    P = jnp.where(row <= col, P, 0.0)
                ps = jnp.sum(P.reshape(16, 8, 128), axis=0)
                ls[j] = ps if ls[j] is None else ls[j] + ps
                O = _dot(vtg[32 * j:32 * j + 32, 128 * t:128 * (t + 1)], P.astype(BF))
                accs[j] = O if accs[j] is None else accs[j] + O
            if t == i:
                nd, gates = mem[gg]
                rows = []
                for j in range(4):
                    l = jnp.sum(ls[j], axis=0, keepdims=True)
                    flag[0] = jnp.where((l >= L_LO) & (l <= L_HI), flag[0], 1.0)
                    gj = gates[j]
                    den = nd[128 + j:129 + j, 128 * i:128 * (i + 1)] + 1e-6
                    num = nd[32 * j:32 * j + 32, 128 * i:128 * (i + 1)]
                    rows.append(accs[j] * ((1.0 - gj) / l) + num * (gj / den))
                o_s[128 * i:128 * (i + 1), pl.ds(c0, 128)] = jnp.concatenate(rows, axis=0).T.astype(BF)

        pend = []
        seen = set()
        for st in steps:
            if st[0] not in seen:
                seen.add(st[0])
                mem_read(st[0])
            pend.append((st, qk(st)))
            if len(pend) > LA:
                pv(*pend.pop(0))
        upd = list(range(ngroups))
        while pend:
            mem_update(upd.pop(0))
            pv(*pend.pop(0))
        for gg in upd:
            mem_update(gg)
        return flag[0]

    def attention_safe(par):
        def body(n, c):
            g, i = n // 4, n % 4
            c0 = pl.multiple_of(g * 128, 128)
            q0 = pl.multiple_of(i * 128, 128)
            qi = qs[pl.ds(q0, 128), pl.ds(c0, 128)]
            W = jnp.concatenate([_head_mask(qi, j) for j in range(4)], axis=0)
            kr = lax.broadcasted_iota(jnp.int32, (128, 512), 0)
            qc = lax.broadcasted_iota(jnp.int32, (128, 512), 1) & 127

            def logits(t):
                k0 = pl.multiple_of(t * 128, 128)
                St = _dot_nt(ks[pl.ds(k0, 128), pl.ds(c0, 128)], W)
                return St + jnp.where(kr + k0 > qc + q0, MASKV, 0.0), k0

            def pass1(t, m):
                return jnp.maximum(m, jnp.max(logits(t)[0], axis=0, keepdims=True))
            m = lax.fori_loop(0, i + 1, pass1, jnp.full((1, 512), -jnp.inf, F32))

            def pass2(t, carry):
                acc, l = carry
                St, k0 = logits(t)
                P = jnp.exp2(St - m)
                outs = [_dot(vt[g, 32 * j:32 * j + 32, pl.ds(k0, 128)],
                             P[:, 128 * j:128 * (j + 1)].astype(BF)) for j in range(4)]
                return acc + jnp.concatenate(outs, axis=0), l + jnp.sum(P, axis=0, keepdims=True)
            acc, l = lax.fori_loop(0, i + 1, pass2,
                                   (jnp.zeros((128, 128), F32), jnp.zeros((1, 512), F32)))

            nd = _dot_nt(mst[par, g].astype(BF), pq[pl.ds(q0, 128), pl.ds(c0, 128)])
            rows = []
            for j in range(4):
                gj = gtab[pl.ds(4 * g + j, 1), :]
                den = nd[128 + j:129 + j, :] + 1e-6
                rows.append(acc[32 * j:32 * j + 32] * ((1.0 - gj) / l[:, 128 * j:128 * (j + 1)])
                            + nd[32 * j:32 * j + 32] * (gj / den))
            o_s[pl.ds(q0, 128), pl.ds(c0, 128)] = jnp.concatenate(rows, axis=0).T.astype(BF)
            return c
        lax.fori_loop(0, NG * 4, body, 0)

    def layer(ell, carry):
        mst[0] = jnp.zeros((NG, VR, 128), F32)
        xnb[0:RB, :] = _ln(xf[0:RB, :]).astype(BF)

        @pl.when(ell == 0)
        def _():
            cvt(2, 0)
            for c in c_w[:3]:
                c.wait()
            for i in range(3, NB):
                c_xb(i).start()
            for c in c_w[3:5]:
                c.start()

        def seg(s, c):
            r0 = pl.multiple_of(s * L, L)

            def qkv(u, c1):
                offs = [pl.multiple_of(u * RB + ch * QCH, QCH) for ch in range(RB // QCH)]
                xbs = [xnb[pl.ds(r0 + o, QCH), :] for o in offs]
                for o, xb in zip(offs, xbs):
                    v = _dot(xb, wv[...])
                    for g in range(NG):
                        vt[g, 0:128, pl.ds(o, QCH)] = v[:, 128 * g:128 * (g + 1)].T.astype(BF)
                rn = pl.multiple_of(jnp.minimum(r0 + (u + 1) * RB, S - RB), RB)
                xnb[pl.ds(rn, RB), :] = _ln(xf[pl.ds(rn, RB), :]).astype(BF)
                for o, xb in zip(offs, xbs):
                    q = _dot(xb, wq[...])
                    qs[pl.ds(o, QCH), :] = (q * QSCALE).astype(BF)
                    pq[pl.ds(o, QCH), :] = _phi(q).astype(BF)
                for o in offs:
                    k = _dot(xnb[pl.ds(r0 + o, QCH), :], wk[...])
                    ks[pl.ds(o, QCH), :] = k.astype(BF)
                    pk[pl.ds(o, QCH), :] = _phi(k).astype(BF)
                return c1

            lax.fori_loop(0, L // RB, qkv, 0)

            @pl.when((ell == 0) & (s < NSEG - 1))
            def _():
                nb = (s + 1) * (L // RB) + 1
                lax.fori_loop(nb, jnp.minimum(nb + L // RB, NB), cvt, 0)

            par = s % 2
            bad = lax.fori_loop(0, NG // GPI,
                                lambda it, b: attention_groups(it * GPI, GPI, par, b),
                                jnp.zeros((1, 128), F32))

            @pl.when(jnp.max(bad) > 0.0)
            def _():
                attention_safe(par)

            @pl.when(jnp.logical_and(ell == 0, s == 0))
            def _():
                for cw in c_w[3:5]:
                    cw.wait()
                for cw in c_w[5:]:
                    cw.start()

            def proj(u, c3):
                offs = [pl.multiple_of(u * RB + ch * PCH, PCH) for ch in range(RB // PCH)]
                xs = []
                for o in offs:
                    x = xf[pl.ds(r0 + o, PCH), :] + _dot(o_s[pl.ds(o, PCH), :], wo[...])
                    xf[pl.ds(r0 + o, PCH), :] = x
                    xs.append(x)
                for o, x in zip(offs, xs):
                    xn = _ln(x)
                    xn_s[pl.ds(r0 + o, PCH), :] = xn
                    h_s[pl.ds(pl.multiple_of(r0 + o + HPAD, 8), PCH), :] = _gelu(_dot(_ln(xn).astype(BF), w1[...]))
                return c3
            lax.fori_loop(0, L // RB, proj, 0)
            return c
        lax.fori_loop(0, NSEG, seg, 0)

        @pl.when(ell == 0)
        def _():
            for cw in c_w[5:]:
                cw.wait()

        def blk(s, c):
            r0 = pl.multiple_of(s * RB, RB)
            offs = [pl.multiple_of(r0 + ch * BCH, BCH) for ch in range(RB // BCH)]
            c4 = D // 4
            hss = []
            for rr in offs:
                parts = []
                for ci, sh in enumerate((-1, 1, -2, 2)):
                    w0 = rr if sh < 0 else rr + HPAD
                    win = h_s[pl.ds(pl.multiple_of(w0, 8), BCH + HPAD), ci * c4:(ci + 1) * c4]
                    o0 = HPAD + sh if sh < 0 else sh
                    parts.append(win[o0:o0 + BCH].astype(BF))
                hss.append(_dot(jnp.concatenate(parts, axis=1), w2[...]))
            for rr, hs in zip(offs, hss):
                x1 = xn_s[pl.ds(rr, BCH), :] + hs
                x1n = _ln(x1).astype(BF)
                acc = xf[pl.ds(rr, BCH), :] + x1
                for f in range(F // FC):
                    hh = _gelu(_dot(x1n, w3[:, f * FC:(f + 1) * FC])).astype(BF)
                    acc = acc + _dot(hh, w4[f * FC:(f + 1) * FC, :])
                xf[pl.ds(rr, BCH), :] = acc
                xio[pl.ds(rr, BCH), :] = acc.astype(BF)

            @pl.when(ell == 1)
            def _():
                pltpu.make_async_copy(xio.at[pl.ds(r0, RB)], out_hbm.at[0, pl.ds(r0, RB)], osem.at[s]).start()
            return c
        lax.fori_loop(0, S // RB, blk, 0)
        return carry

    lax.fori_loop(0, 2, layer, 0)
    for s in range(S // RB):
        pltpu.make_async_copy(xio.at[pl.ds(s * RB, RB)], out_hbm.at[0, pl.ds(s * RB, RB)], osem.at[s]).wait()


@jax.jit
def pallas_interleave_layers__memory_aug_infini_attn__mixer_s_mlp__prompt_kernel(
    A_x, A_wq, A_wk, A_wv, A_wo, A_beta, B_x, B_w1, B_w2, B_w3, B_w4,
):
    del B_x
    any_spec = pl.BlockSpec(memory_space=pl.ANY)
    vm = pltpu.VMEM
    scratch = [
        vm((D, D), BF), vm((D, D), BF), vm((D, D), BF), vm((D, D), BF),
        vm((D, D), BF), vm((D, D), BF), vm((D, F), BF), vm((F, D), BF),
        vm((S, D), F32), vm((S, D), F32), vm((S + 2 * HPAD, D), F32),
        vm((S, D), BF), vm((S, D), BF),
        vm((L, D), BF), vm((L, D), BF), vm((L, D), BF), vm((L, D), BF),
        vm((NG, VR, L), BF), vm((L, D), BF),
        vm((2, NG, VR, 128), F32), vm((H, 128), F32),
        pltpu.SemaphoreType.DMA((9 + S // RB,)), pltpu.SemaphoreType.DMA((8,)),
    ]
    return pl.pallas_call(
        _kernel,
        out_shape=jax.ShapeDtypeStruct((1, S, D), BF),
        in_specs=[pl.BlockSpec(memory_space=pltpu.VMEM)] + [any_spec] * 9,
        out_specs=any_spec,
        scratch_shapes=scratch,
        compiler_params=pltpu.CompilerParams(vmem_limit_bytes=110 * 2 ** 20),
        name="fused_infini_mixer",
    )(A_beta.reshape(1, H), A_x, A_wq, A_wk, A_wv, A_wo, B_w1, B_w2, B_w3, B_w4)
```

```python
import functools

import numpy as np
import jax
import jax.numpy as jnp
from jax import lax
import jax.experimental.pallas as pl
import jax.experimental.pallas.tpu as pltpu

S, D, H, DH, NSEG, L, F = 2048, 1024, 32, 32, 4, 512, 3584
NG = D // 128
BF, F32 = jnp.bfloat16, jnp.float32
NT = (((1,), (1,)), ((), ()))
EPS = 1e-5
LOG2E = float(np.log2(np.e))
QSCALE = float(DH ** -0.5) * LOG2E
GC = float(np.sqrt(2.0 / np.pi))
HPAD = 8
L_LO, L_HI = 2.0 ** -40, 2.0 ** 40
MASKV = -1e9 * LOG2E
GPI = 4
LA = 2
RB = 256
PCH, BCH = 128, 128
FC = 896
VR = 144


def _ln(x):
    m = jnp.mean(x, axis=-1, keepdims=True)
    xc = x - m
    v = jnp.mean(xc * xc, axis=-1, keepdims=True)
    return xc * lax.rsqrt(v + EPS)


def _gelu(x):
    return 0.5 * x * (1.0 + jnp.tanh(GC * (x + 0.044715 * (x * x * x))))


def _phi(x):
    return jnp.where(x > 0, x + 1.0, jnp.exp(x))


def _dot(a, b):
    return jnp.dot(a, b, preferred_element_type=F32)


def _dot_nt(a, b):
    return lax.dot_general(a, b, NT, preferred_element_type=F32)


def _head_mask(x, j):
    lane = lax.broadcasted_iota(jnp.int32, (1, 128), 1)
    m = jnp.where((lane >= 32 * j) & (lane < 32 * j + 32), -1, 0).astype(jnp.int32)
    return pltpu.bitcast(pltpu.bitcast(x, jnp.int32) & m, BF)


def _kernel(beta_ref, x_hbm, wq_hbm, wk_hbm, wv_hbm, wo_hbm, w1_hbm, w2_hbm, w3_hbm, w4_hbm,
            out_hbm,
            wq, wk, wv, wo, w1, w2, w3, w4,
            xf, xn_s, h_s, xio, xnb, qs, pq, ks, pk, vt, o_s, mst, gtab, sem, osem, qsem):
    def cp(src, dst, i):
        return pltpu.make_async_copy(src, dst, sem.at[i])
    NB = S // RB

    def c_xb(i):
        r = pl.multiple_of(i * RB, RB)
        return cp(x_hbm.at[0, pl.ds(r, RB)], xio.at[pl.ds(r, RB)], 9 + i)
    WC = GPI * 128

    def c_qkv(j):
        c = pl.multiple_of(j * WC, WC)
        return [pltpu.make_async_copy(src.at[:, pl.ds(c, WC)], dst.at[:, pl.ds(c, WC)], qsem.at[j, m])
                for m, (src, dst) in enumerate(((wv_hbm, wv), (wq_hbm, wq), (wk_hbm, wk)))]
    c_w = [cp(wo_hbm, wo, 4), cp(w1_hbm, w1, 5), cp(w2_hbm, w2, 6), cp(w3_hbm, w3, 7), cp(w4_hbm, w4, 8)]
    assert NG // GPI == 2 and L // RB == 2
    for c in [c_xb(0), c_xb(1), c_xb(2)] + c_qkv(0):
        c.start()

    b = beta_ref[...].astype(F32)
    hrow = lax.broadcasted_iota(jnp.int32, (H, H), 0)
    hcol = lax.broadcasted_iota(jnp.int32, (H, H), 1)
    bcol = jnp.sum(jnp.where(hrow == hcol, jnp.broadcast_to(b, (H, H)), 0.0), axis=1, keepdims=True)
    gtab[...] = jnp.broadcast_to(jax.nn.sigmoid(bcol), (H, 128))

    for g in range(NG):
        vt[g, 128:VR, :] = jnp.ones((VR - 128, L), BF)
    h_s[0:HPAD, :] = jnp.zeros((HPAD, D), F32)
    h_s[HPAD + S:HPAD + S + HPAD, :] = jnp.zeros((HPAD, D), F32)

    def cvt(i, c):
        c_xb(i).wait()
        r = pl.multiple_of(i * RB, RB)
        xf[pl.ds(r, RB), :] = xio[pl.ds(r, RB), :].astype(F32)
        return c
    lax.fori_loop(0, 2, cvt, 0)

    row = lax.broadcasted_iota(jnp.int32, (128, 128), 0)
    col = lax.broadcasted_iota(jnp.int32, (128, 128), 1)

    def attention_groups(g0, ngroups, par, bad, r0, rn):
        flag = [bad]
        steps = [(gg, i, t) for gg in range(ngroups) for i in (3, 2, 1, 0) for t in range(i + 1)]
        ctx, wcache, state, mem = {}, {}, {}, {}

        xb = [xnb[pl.ds(r0, L), :]]

        def project(gg):
            g = g0 + gg
            c0 = pl.multiple_of(g * 128, 128)
            v = _dot(xb[0], wv[:, pl.ds(c0, 128)])
            vt[g, 0:128, :] = v.T.astype(BF)
            q = _dot(xb[0], wq[:, pl.ds(c0, 128)])
            qs[:, pl.ds(c0, 128)] = (q * QSCALE).astype(BF)
            pq[:, pl.ds(c0, 128)] = _phi(q).astype(BF)
            k = _dot(xb[0], wk[:, pl.ds(c0, 128)])
            ks[:, pl.ds(c0, 128)] = k.astype(BF)
            pk[:, pl.ds(c0, 128)] = _phi(k).astype(BF)
            if gg == 1:
                xnb[pl.ds(rn, RB), :] = _ln(xf[pl.ds(rn, RB), :]).astype(BF)
                xb[0] = xnb[pl.ds(r0, L), :]

        def getg(gg):
            if gg not in ctx:
                g = g0 + gg
                c0 = pl.multiple_of(g * 128, 128)
                ctx[gg] = (g, c0, qs[:, pl.ds(c0, 128)], ks[:, pl.ds(c0, 128)], vt[g])
            return ctx[gg]

        def mem_read(gg):
            g, c0, _, _, vtg = getg(gg)
            nd = _dot_nt(mst[par, g].astype(BF), pq[:, pl.ds(c0, 128)])
            gates = [gtab[pl.ds(4 * g + j, 1), :] for j in range(4)]
            mem[gg] = (nd, gates)

        def mem_update(gg):
            g, c0, _, _, vtg = getg(gg)
            upd = _dot(vtg, pk[:, pl.ds(c0, 128)])
            r = lax.broadcasted_iota(jnp.int32, (VR, 128), 0)
            c = lax.broadcasted_iota(jnp.int32, (VR, 128), 1)
            keep = jnp.where(r < 128, r // 32, r - 128) == c // 32
            mst[1 - par, g] = mst[par, g] + jnp.where(keep, upd, 0.0)

        def qk(st):
            gg, i, t = st
            _, _, qg, kg, _ = getg(gg)
            if (gg, i) not in wcache:
                qi = qg[128 * i:128 * (i + 1)]
                wcache[(gg, i)] = jnp.concatenate([_head_mask(qi, j) for j in range(4)], axis=0)
            return _dot_nt(kg[128 * t:128 * (t + 1)], wcache[(gg, i)])

        def pv(st, St):
            gg, i, t = st
            g, c0, _, _, vtg = getg(gg)
            accs, ls = state.setdefault((gg, i), ([None] * 4, [None] * 4))
            for j in range(4):
                P = jnp.exp2(St[:, 128 * j:128 * (j + 1)])
                if t == i:
                    P = jnp.where(row <= col, P, 0.0)
                ps = jnp.sum(P.reshape(16, 8, 128), axis=0)
                ls[j] = ps if ls[j] is None else ls[j] + ps
                O = _dot(vtg[32 * j:32 * j + 32, 128 * t:128 * (t + 1)], P.astype(BF))
                accs[j] = O if accs[j] is None else accs[j] + O
            if t == i:
                nd, gates = mem[gg]
                rows = []
                for j in range(4):
                    l = jnp.sum(ls[j], axis=0, keepdims=True)
                    flag[0] = jnp.where((l >= L_LO) & (l <= L_HI), flag[0], 1.0)
                    gj = gates[j]
                    den = nd[128 + j:129 + j, 128 * i:128 * (i + 1)] + 1e-6
                    num = nd[32 * j:32 * j + 32, 128 * i:128 * (i + 1)]
                    rows.append(accs[j] * ((1.0 - gj) / l) + num * (gj / den))
                o_s[128 * i:128 * (i + 1), pl.ds(c0, 128)] = jnp.concatenate(rows, axis=0).T.astype(BF)

        pend = []
        seen = set()
        project(0)
        for st in steps:
            if st[0] not in seen:
                seen.add(st[0])
                if st[0] + 1 < ngroups:
                    project(st[0] + 1)
                mem_read(st[0])
            pend.append((st, qk(st)))
            if len(pend) > LA:
                pv(*pend.pop(0))
        upd = list(range(ngroups))
        while pend:
            mem_update(upd.pop(0))
            pv(*pend.pop(0))
        for gg in upd:
            mem_update(gg)
        return flag[0]

    def attention_safe(par):
        def body(n, c):
            g, i = n // 4, n % 4
            c0 = pl.multiple_of(g * 128, 128)
            q0 = pl.multiple_of(i * 128, 128)
            qi = qs[pl.ds(q0, 128), pl.ds(c0, 128)]
            W = jnp.concatenate([_head_mask(qi, j) for j in range(4)], axis=0)
            kr = lax.broadcasted_iota(jnp.int32, (128, 512), 0)
            qc = lax.broadcasted_iota(jnp.int32, (128, 512), 1) & 127

            def logits(t):
                k0 = pl.multiple_of(t * 128, 128)
                St = _dot_nt(ks[pl.ds(k0, 128), pl.ds(c0, 128)], W)
                return St + jnp.where(kr + k0 > qc + q0, MASKV, 0.0), k0

            def pass1(t, m):
                return jnp.maximum(m, jnp.max(logits(t)[0], axis=0, keepdims=True))
            m = lax.fori_loop(0, i + 1, pass1, jnp.full((1, 512), -jnp.inf, F32))

            def pass2(t, carry):
                acc, l = carry
                St, k0 = logits(t)
                P = jnp.exp2(St - m)
                outs = [_dot(vt[g, 32 * j:32 * j + 32, pl.ds(k0, 128)],
                             P[:, 128 * j:128 * (j + 1)].astype(BF)) for j in range(4)]
                return acc + jnp.concatenate(outs, axis=0), l + jnp.sum(P, axis=0, keepdims=True)
            acc, l = lax.fori_loop(0, i + 1, pass2,
                                   (jnp.zeros((128, 128), F32), jnp.zeros((1, 512), F32)))

            nd = _dot_nt(mst[par, g].astype(BF), pq[pl.ds(q0, 128), pl.ds(c0, 128)])
            rows = []
            for j in range(4):
                gj = gtab[pl.ds(4 * g + j, 1), :]
                den = nd[128 + j:129 + j, :] + 1e-6
                rows.append(acc[32 * j:32 * j + 32] * ((1.0 - gj) / l[:, 128 * j:128 * (j + 1)])
                            + nd[32 * j:32 * j + 32] * (gj / den))
            o_s[pl.ds(q0, 128), pl.ds(c0, 128)] = jnp.concatenate(rows, axis=0).T.astype(BF)
            return c
        lax.fori_loop(0, NG * 4, body, 0)

    def layer(ell, carry):
        mst[0] = jnp.zeros((NG, VR, 128), F32)

        def ln0(i, c):
            r = pl.multiple_of(i * RB, RB)
            xnb[pl.ds(r, RB), :] = _ln(xf[pl.ds(r, RB), :]).astype(BF)
            return c
        lax.fori_loop(0, L // RB, ln0, 0)

        def seg(s, c):
            r0 = pl.multiple_of(s * L, L)
            par = s % 2

            def qa(j, bad):
                nb = (s + 1) * (L // RB) + j

                @pl.when(ell == 0)
                def _():
                    @pl.when(nb < NB)
                    def _():
                        cvt(nb, 0)

                    @pl.when(s == 0)
                    def _():
                        for cw in c_qkv(j):
                            cw.wait()

                        @pl.when(j == 0)
                        def _():
                            for cw in [c_xb(3)] + c_qkv(1):
                                cw.start()

                        @pl.when(j == 1)
                        def _():
                            for cw in c_w[:2] + [c_xb(i) for i in range(4, NB)]:
                                cw.start()
                rn = pl.multiple_of(jnp.minimum(nb, NB - 1) * RB, RB)
                return attention_groups(j * GPI, GPI, par, bad, r0, rn)
            bad = lax.fori_loop(0, NG // GPI, qa, jnp.zeros((1, 128), F32))

            @pl.when(jnp.max(bad) > 0.0)
            def _():
                attention_safe(par)

            @pl.when(jnp.logical_and(ell == 0, s == 0))
            def _():
                for cw in c_w[:2]:
                    cw.wait()
                for cw in c_w[2:]:
                    cw.start()

            def proj(u, c3):
                offs = [pl.multiple_of(u * RB + ch * PCH, PCH) for ch in range(RB // PCH)]
                xs = []
                for o in offs:
                    x = xf[pl.ds(r0 + o, PCH), :] + _dot(o_s[pl.ds(o, PCH), :], wo[...])
                    xf[pl.ds(r0 + o, PCH), :] = x
                    xs.append(x)
                for o, x in zip(offs, xs):
                    xn = _ln(x)
                    xn_s[pl.ds(r0 + o, PCH), :] = xn
                    h_s[pl.ds(pl.multiple_of(r0 + o + HPAD, 8), PCH), :] = _gelu(_dot(_ln(xn).astype(BF), w1[...]))
                return c3
            lax.fori_loop(0, L // RB, proj, 0)
            return c
        lax.fori_loop(0, NSEG, seg, 0)

        @pl.when(ell == 0)
        def _():
            for cw in c_w[2:]:
                cw.wait()

        def blk(s, c):
            r0 = pl.multiple_of(s * RB, RB)
            offs = [pl.multiple_of(r0 + ch * BCH, BCH) for ch in range(RB // BCH)]
            c4 = D // 4
            hss = []
            for rr in offs:
                parts = []
                for ci, sh in enumerate((-1, 1, -2, 2)):
                    w0 = rr if sh < 0 else rr + HPAD
                    win = h_s[pl.ds(pl.multiple_of(w0, 8), BCH + HPAD), ci * c4:(ci + 1) * c4]
                    o0 = HPAD + sh if sh < 0 else sh
                    parts.append(win[o0:o0 + BCH].astype(BF))
                hss.append(_dot(jnp.concatenate(parts, axis=1), w2[...]))
            for rr, hs in zip(offs, hss):
                x1 = xn_s[pl.ds(rr, BCH), :] + hs
                x1n = _ln(x1).astype(BF)
                acc = xf[pl.ds(rr, BCH), :] + x1
                for f in range(F // FC):
                    hh = _gelu(_dot(x1n, w3[:, f * FC:(f + 1) * FC])).astype(BF)
                    acc = acc + _dot(hh, w4[f * FC:(f + 1) * FC, :])
                xf[pl.ds(rr, BCH), :] = acc
                xio[pl.ds(rr, BCH), :] = acc.astype(BF)

            @pl.when(ell == 1)
            def _():
                pltpu.make_async_copy(xio.at[pl.ds(r0, RB)], out_hbm.at[0, pl.ds(r0, RB)], osem.at[s]).start()
            return c
        lax.fori_loop(0, S // RB, blk, 0)
        return carry

    lax.fori_loop(0, 2, layer, 0)
    for s in range(S // RB):
        pltpu.make_async_copy(xio.at[pl.ds(s * RB, RB)], out_hbm.at[0, pl.ds(s * RB, RB)], osem.at[s]).wait()


@jax.jit
def pallas_interleave_layers__memory_aug_infini_attn__mixer_s_mlp__prompt_kernel(
    A_x, A_wq, A_wk, A_wv, A_wo, A_beta, B_x, B_w1, B_w2, B_w3, B_w4,
):
    del B_x
    any_spec = pl.BlockSpec(memory_space=pl.ANY)
    vm = pltpu.VMEM
    scratch = [
        vm((D, D), BF), vm((D, D), BF), vm((D, D), BF), vm((D, D), BF),
        vm((D, D), BF), vm((D, D), BF), vm((D, F), BF), vm((F, D), BF),
        vm((S, D), F32), vm((S, D), F32), vm((S + 2 * HPAD, D), F32),
        vm((S, D), BF), vm((S, D), BF),
        vm((L, D), BF), vm((L, D), BF), vm((L, D), BF), vm((L, D), BF),
        vm((NG, VR, L), BF), vm((L, D), BF),
        vm((2, NG, VR, 128), F32), vm((H, 128), F32),
        pltpu.SemaphoreType.DMA((9 + S // RB,)), pltpu.SemaphoreType.DMA((8,)),
        pltpu.SemaphoreType.DMA((NG // GPI, 3)),
    ]
    return pl.pallas_call(
        _kernel,
        out_shape=jax.ShapeDtypeStruct((1, S, D), BF),
        in_specs=[pl.BlockSpec(memory_space=pltpu.VMEM)] + [any_spec] * 9,
        out_specs=any_spec,
        scratch_shapes=scratch,
        compiler_params=pltpu.CompilerParams(vmem_limit_bytes=110 * 2 ** 20),
        name="fused_infini_mixer",
    )(A_beta.reshape(1, H), A_x, A_wq, A_wk, A_wv, A_wo, B_w1, B_w2, B_w3, B_w4)
```

```python
import functools

import numpy as np
import jax
import jax.numpy as jnp
from jax import lax
import jax.experimental.pallas as pl
import jax.experimental.pallas.tpu as pltpu

S, D, H, DH, NSEG, L, F = 2048, 1024, 32, 32, 4, 512, 3584
NG = D // 128
BF, F32 = jnp.bfloat16, jnp.float32
NT = (((1,), (1,)), ((), ()))
EPS = 1e-5
LOG2E = float(np.log2(np.e))
QSCALE = float(DH ** -0.5) * LOG2E
GC = float(np.sqrt(2.0 / np.pi))
HPAD = 8
L_LO, L_HI = 2.0 ** -40, 2.0 ** 40
MASKV = -1e9 * LOG2E
GPI = 4
LA = 2
LS = 0
NPR = 1
PPOS = (0, 0, 0)
MPOS = 0
PAH = 1
LNG = 1
DFIRST = 0
IORD = (0, 3, 2, 1)
RB = 256
PRB = 256
PCH, BCH = 128, 128
FC = 896
VR = 144


def _ln(x):
    m = jnp.mean(x, axis=-1, keepdims=True)
    xc = x - m
    v = jnp.mean(xc * xc, axis=-1, keepdims=True)
    return xc * lax.rsqrt(v + EPS)


def _gelu(x):
    return 0.5 * x * (1.0 + jnp.tanh(GC * (x + 0.044715 * (x * x * x))))


def _phi(x):
    return jnp.where(x > 0, x + 1.0, jnp.exp(x))


def _dot(a, b):
    return jnp.dot(a, b, preferred_element_type=F32)


def _dot_nt(a, b):
    return lax.dot_general(a, b, NT, preferred_element_type=F32)


def _head_mask(x, j):
    lane = lax.broadcasted_iota(jnp.int32, (1, 128), 1)
    m = jnp.where((lane >= 32 * j) & (lane < 32 * j + 32), -1, 0).astype(jnp.int32)
    return pltpu.bitcast(pltpu.bitcast(x, jnp.int32) & m, BF)


def _kernel(beta_ref, x_hbm, wq_hbm, wk_hbm, wv_hbm, wo_hbm, w1_hbm, w2_hbm, w3_hbm, w4_hbm,
            out_hbm,
            wq, wk, wv, wo, w1, w2, w3, w4,
            xf, xn_s, h_s, xio, xnb, qs, pq, ks, pk, vt, o_s, mst, gtab, mtab, sem, osem, qsem):
    def cp(src, dst, i):
        return pltpu.make_async_copy(src, dst, sem.at[i])
    NB = S // RB

    def c_xb(i):
        r = pl.multiple_of(i * RB, RB)
        return cp(x_hbm.at[0, pl.ds(r, RB)], xio.at[pl.ds(r, RB)], 9 + i)
    WC = GPI * 128

    def c_qkv(j):
        c = pl.multiple_of(j * WC, WC)
        return [pltpu.make_async_copy(src.at[:, pl.ds(c, WC)], dst.at[:, pl.ds(c, WC)], qsem.at[j, m])
                for m, (src, dst) in enumerate(((wv_hbm, wv), (wq_hbm, wq), (wk_hbm, wk)))]
    c_w = [cp(wo_hbm, wo, 4), cp(w1_hbm, w1, 5), cp(w2_hbm, w2, 6), cp(w3_hbm, w3, 7), cp(w4_hbm, w4, 8)]
    assert NG // GPI == 2 and L // RB == 2
    for c in [c_xb(0), c_xb(1), c_xb(2)] + c_qkv(0):
        c.start()

    b = beta_ref[...].astype(F32)
    hrow = lax.broadcasted_iota(jnp.int32, (H, H), 0)
    hcol = lax.broadcasted_iota(jnp.int32, (H, H), 1)
    bcol = jnp.sum(jnp.where(hrow == hcol, jnp.broadcast_to(b, (H, H)), 0.0), axis=1, keepdims=True)
    gtab[...] = jnp.broadcast_to(jax.nn.sigmoid(bcol), (H, 128))

    mr = lax.broadcasted_iota(jnp.int32, (128, 128), 0)
    mc = lax.broadcasted_iota(jnp.int32, (128, 128), 1)
    mtab[0] = jnp.where(mr <= (mc ^ 64), jnp.inf, 0.0)
    mtab[1] = jnp.where(mr <= mc, jnp.inf, 0.0)
    for g in range(NG):
        vt[g, 128:VR, :] = jnp.ones((VR - 128, L), BF)
    h_s[0:HPAD, :] = jnp.zeros((HPAD, D), F32)
    h_s[HPAD + S:HPAD + S + HPAD, :] = jnp.zeros((HPAD, D), F32)

    def cvt(i, c):
        c_xb(i).wait()
        r = pl.multiple_of(i * RB, RB)
        xf[pl.ds(r, RB), :] = xio[pl.ds(r, RB), :].astype(F32)
        return c
    lax.fori_loop(0, 2, cvt, 0)

    row = lax.broadcasted_iota(jnp.int32, (128, 128), 0)
    col = lax.broadcasted_iota(jnp.int32, (128, 128), 1)

    def attention_groups(g0, ngroups, par, bad, r0, rn):
        flag = [bad]
        steps = [(gg, i, t) for gg in range(ngroups) for i in IORD
                 for t in (range(i, -1, -1) if DFIRST else range(i + 1))]
        ctx, wcache, state, mem = {}, {}, {}, {}

        xb = [xnb[pl.ds(r0, L), :]]

        def project(gg, piece):
            g = g0 + gg
            c0 = pl.multiple_of(g * 128, 128)
            which, rc = divmod(piece, NPR)
            n = L // NPR
            x = xb[0][rc * n:(rc + 1) * n]
            rows = slice(rc * n, (rc + 1) * n)
            if which == 0:
                v = _dot(x, wv[:, pl.ds(c0, 128)])
                vt[g, 0:128, rows] = v.T.astype(BF)
            elif which == 1:
                q = _dot(x, wq[:, pl.ds(c0, 128)])
                qs[rows, pl.ds(c0, 128)] = (q * QSCALE).astype(BF)
                pq[rows, pl.ds(c0, 128)] = _phi(q).astype(BF)
            else:
                k = _dot(x, wk[:, pl.ds(c0, 128)])
                ks[rows, pl.ds(c0, 128)] = k.astype(BF)
                pk[rows, pl.ds(c0, 128)] = _phi(k).astype(BF)
                if gg == LNG and rc == NPR - 1:
                    xnb[pl.ds(rn, RB), :] = _ln(xf[pl.ds(rn, RB), :]).astype(BF)
                    xb[0] = xnb[pl.ds(r0, L), :]

        def getg(gg):
            if gg not in ctx:
                g = g0 + gg
                c0 = pl.multiple_of(g * 128, 128)
                ctx[gg] = (g, c0, qs[:, pl.ds(c0, 128)], ks[:, pl.ds(c0, 128)], vt[g])
            return ctx[gg]

        def mem_read(gg):
            g, c0, _, _, vtg = getg(gg)
            nd = _dot_nt(mst[par, g].astype(BF), pq[:, pl.ds(c0, 128)])
            gates = [gtab[pl.ds(4 * g + j, 1), :] for j in range(4)]
            mem[gg] = (nd, gates)

        def mem_update(gg):
            g, c0, _, _, vtg = getg(gg)
            upd = _dot(vtg, pk[:, pl.ds(c0, 128)])
            r = lax.broadcasted_iota(jnp.int32, (VR, 128), 0)
            c = lax.broadcasted_iota(jnp.int32, (VR, 128), 1)
            keep = jnp.where(r < 128, r // 32, r - 128) == c // 32
            mst[1 - par, g] = mst[par, g] + jnp.where(keep, upd, 0.0)

        def qk(st):
            gg, i, t = st
            _, _, qg, kg, _ = getg(gg)
            if (gg, i) not in wcache:
                lo, hi = qg[128 * i:128 * i + 64], qg[128 * i + 64:128 * (i + 1)]
                ms = [_head_mask(jnp.concatenate([lo, hi] if j % 2 else [hi, lo], axis=0), j)
                      for j in range(4)]
                wcache[(gg, i)] = (jnp.concatenate(ms, axis=0),
                                   jnp.concatenate([ms[0][:64], ms[1][64:], ms[2][:64], ms[3][64:]], axis=0))
            W, Whi = wcache[(gg, i)]
            if t < i:
                return _dot_nt(kg[128 * t:128 * (t + 1)], W)
            return (_dot_nt(kg[128 * t:128 * t + 64], W),
                    _dot_nt(kg[128 * t + 64:128 * (t + 1)], Whi))

        def probs(St, j):
            if not isinstance(St, tuple):
                return jnp.exp2(St[:, 128 * j:128 * (j + 1)])
            Slo, Shi = St
            r = lax.broadcasted_iota(jnp.int32, (64, 128), 0)
            c = lax.broadcasted_iota(jnp.int32, (64, 128), 1)
            qi = c if j % 2 else c ^ 64
            plo = jnp.minimum(jnp.exp2(Slo[:, 128 * j:128 * (j + 1)]), mtab[j % 2, 0:64])
            phi = jnp.minimum(Ehi[j // 2], mtab[j % 2, 64:128])
            return jnp.concatenate([plo, phi], axis=0)

        Ehi = [None, None]

        def softmax_tile(st, St):
            gg, i, t = st
            accs, ls = state.setdefault((gg, i), ([None] * 4, [None] * 4))
            if isinstance(St, tuple):
                Ehi[:] = [jnp.exp2(St[1][:, :128]), jnp.exp2(St[1][:, 128:])]
            out = []
            for j in range(4):
                P = probs(St, j)
                ps = jnp.sum(P.reshape(16, 8, 128), axis=0)
                ls[j] = ps if ls[j] is None else ls[j] + ps
                out.append(P.astype(BF))
            return out

        def pv(st, Pb):
            gg, i, t = st
            g, c0, _, _, vtg = getg(gg)
            accs, ls = state[(gg, i)]
            for j in range(4):
                O = _dot(vtg[32 * j:32 * j + 32, 128 * t:128 * (t + 1)], Pb[j])
                accs[j] = O if accs[j] is None else accs[j] + O
            if t == (0 if DFIRST else i):
                nd, gates = mem[gg]
                rows = []
                for j in range(4):
                    l = jnp.sum(ls[j], axis=0, keepdims=True)
                    flag[0] = jnp.where((l >= L_LO) & (l <= L_HI), flag[0], 1.0)
                    gj = gates[j]
                    den = nd[128 + j:129 + j, 128 * i:128 * (i + 1)] + 1e-6
                    num = nd[32 * j:32 * j + 32, 128 * i:128 * (i + 1)]
                    dot = accs[j] * ((1.0 - gj) / l)
                    if j % 2 == 0:
                        dot = pltpu.roll(dot, 64, 1)
                    rows.append(dot + num * (gj / den))
                o_s[128 * i:128 * (i + 1), pl.ds(c0, 128)] = jnp.concatenate(rows, axis=0).T.astype(BF)

        pend, spend = [], []
        for gg in range(PAH):
            for piece in range(3 * NPR):
                project(gg, piece)
        for n, st in enumerate(steps):
            gg, pos = divmod(n, 10)
            if gg + PAH < ngroups:
                for piece in range(3 * NPR):
                    if PPOS[piece] == pos:
                        project(gg + PAH, piece)
            if pos == MPOS:
                mem_read(gg)
            spend.append((st, qk(st)))
            if len(spend) > LS:
                pend.append((spend[0][0], softmax_tile(*spend.pop(0))))
            if len(pend) > LA - LS:
                pv(*pend.pop(0))
        upd = list(range(ngroups))
        while spend:
            pend.append((spend[0][0], softmax_tile(*spend.pop(0))))
        while pend:
            mem_update(upd.pop(0))
            pv(*pend.pop(0))
        for gg in upd:
            mem_update(gg)
        return flag[0]

    def attention_safe(par):
        def body(n, c):
            g, i = n // 4, n % 4
            c0 = pl.multiple_of(g * 128, 128)
            q0 = pl.multiple_of(i * 128, 128)
            qi = qs[pl.ds(q0, 128), pl.ds(c0, 128)]
            W = jnp.concatenate([_head_mask(qi, j) for j in range(4)], axis=0)
            kr = lax.broadcasted_iota(jnp.int32, (128, 512), 0)
            qc = lax.broadcasted_iota(jnp.int32, (128, 512), 1) & 127

            def logits(t):
                k0 = pl.multiple_of(t * 128, 128)
                St = _dot_nt(ks[pl.ds(k0, 128), pl.ds(c0, 128)], W)
                return St + jnp.where(kr + k0 > qc + q0, MASKV, 0.0), k0

            def pass1(t, m):
                return jnp.maximum(m, jnp.max(logits(t)[0], axis=0, keepdims=True))
            m = lax.fori_loop(0, i + 1, pass1, jnp.full((1, 512), -jnp.inf, F32))

            def pass2(t, carry):
                acc, l = carry
                St, k0 = logits(t)
                P = jnp.exp2(St - m)
                outs = [_dot(vt[g, 32 * j:32 * j + 32, pl.ds(k0, 128)],
                             P[:, 128 * j:128 * (j + 1)].astype(BF)) for j in range(4)]
                return acc + jnp.concatenate(outs, axis=0), l + jnp.sum(P, axis=0, keepdims=True)
            acc, l = lax.fori_loop(0, i + 1, pass2,
                                   (jnp.zeros((128, 128), F32), jnp.zeros((1, 512), F32)))

            nd = _dot_nt(mst[par, g].astype(BF), pq[pl.ds(q0, 128), pl.ds(c0, 128)])
            rows = []
            for j in range(4):
                gj = gtab[pl.ds(4 * g + j, 1), :]
                den = nd[128 + j:129 + j, :] + 1e-6
                rows.append(acc[32 * j:32 * j + 32] * ((1.0 - gj) / l[:, 128 * j:128 * (j + 1)])
                            + nd[32 * j:32 * j + 32] * (gj / den))
            o_s[pl.ds(q0, 128), pl.ds(c0, 128)] = jnp.concatenate(rows, axis=0).T.astype(BF)
            return c
        lax.fori_loop(0, NG * 4, body, 0)

    def layer(ell, carry):
        mst[0] = jnp.zeros((NG, VR, 128), F32)

        def ln0(i, c):
            r = pl.multiple_of(i * RB, RB)
            xnb[pl.ds(r, RB), :] = _ln(xf[pl.ds(r, RB), :]).astype(BF)
            return c
        lax.fori_loop(0, L // RB, ln0, 0)

        def seg(s, c):
            r0 = pl.multiple_of(s * L, L)
            par = s % 2

            def qa(j, bad):
                nb = (s + 1) * (L // RB) + j

                @pl.when(ell == 0)
                def _():
                    @pl.when(nb < NB)
                    def _():
                        cvt(nb, 0)

                    @pl.when(s == 0)
                    def _():
                        for cw in c_qkv(j):
                            cw.wait()

                        @pl.when(j == 0)
                        def _():
                            for cw in [c_xb(3)] + c_qkv(1):
                                cw.start()

                        @pl.when(j == 1)
                        def _():
                            for cw in c_w[:2] + [c_xb(i) for i in range(4, NB)]:
                                cw.start()
                rn = pl.multiple_of(jnp.minimum(nb, NB - 1) * RB, RB)
                return attention_groups(j * GPI, GPI, par, bad, r0, rn)
            bad = lax.fori_loop(0, NG // GPI, qa, jnp.zeros((1, 128), F32))

            @pl.when(jnp.max(bad) > 0.0)
            def _():
                attention_safe(par)

            @pl.when(jnp.logical_and(ell == 0, s == 0))
            def _():
                for cw in c_w[:2]:
                    cw.wait()
                for cw in c_w[2:]:
                    cw.start()

            def proj(u, c3):
                offs = [pl.multiple_of(u * PRB + ch * PCH, PCH) for ch in range(PRB // PCH)]
                xs = []
                for o in offs:
                    x = xf[pl.ds(r0 + o, PCH), :] + _dot(o_s[pl.ds(o, PCH), :], wo[...])
                    xf[pl.ds(r0 + o, PCH), :] = x
                    xs.append(x)
                for o, x in zip(offs, xs):
                    xn = _ln(x)
                    xn_s[pl.ds(r0 + o, PCH), :] = xn
                    h_s[pl.ds(pl.multiple_of(r0 + o + HPAD, 8), PCH), :] = _gelu(_dot(_ln(xn).astype(BF), w1[...]))
                return c3
            lax.fori_loop(0, L // PRB, proj, 0)
            return c
        lax.fori_loop(0, NSEG, seg, 0)

        @pl.when(ell == 0)
        def _():
            for cw in c_w[2:]:
                cw.wait()

        def blk(s, c):
            r0 = pl.multiple_of(s * RB, RB)
            offs = [pl.multiple_of(r0 + ch * BCH, BCH) for ch in range(RB // BCH)]
            c4 = D // 4
            hss = []
            for rr in offs:
                parts = []
                for ci, sh in enumerate((-1, 1, -2, 2)):
                    w0 = rr if sh < 0 else rr + HPAD
                    win = h_s[pl.ds(pl.multiple_of(w0, 8), BCH + HPAD), ci * c4:(ci + 1) * c4]
                    o0 = HPAD + sh if sh < 0 else sh
                    parts.append(win[o0:o0 + BCH].astype(BF))
                hss.append(_dot(jnp.concatenate(parts, axis=1), w2[...]))
            for rr, hs in zip(offs, hss):
                x1 = xn_s[pl.ds(rr, BCH), :] + hs
                x1n = _ln(x1).astype(BF)
                acc = xf[pl.ds(rr, BCH), :] + x1
                for f in range(F // FC):
                    hh = _gelu(_dot(x1n, w3[:, f * FC:(f + 1) * FC])).astype(BF)
                    acc = acc + _dot(hh, w4[f * FC:(f + 1) * FC, :])
                xf[pl.ds(rr, BCH), :] = acc
                xio[pl.ds(rr, BCH), :] = acc.astype(BF)

            @pl.when(ell == 1)
            def _():
                pltpu.make_async_copy(xio.at[pl.ds(r0, RB)], out_hbm.at[0, pl.ds(r0, RB)], osem.at[s]).start()
            return c
        lax.fori_loop(0, S // RB, blk, 0)
        return carry

    lax.fori_loop(0, 2, layer, 0)
    for s in range(S // RB):
        pltpu.make_async_copy(xio.at[pl.ds(s * RB, RB)], out_hbm.at[0, pl.ds(s * RB, RB)], osem.at[s]).wait()


@jax.jit
def pallas_interleave_layers__memory_aug_infini_attn__mixer_s_mlp__prompt_kernel(
    A_x, A_wq, A_wk, A_wv, A_wo, A_beta, B_x, B_w1, B_w2, B_w3, B_w4,
):
    del B_x
    any_spec = pl.BlockSpec(memory_space=pl.ANY)
    vm = pltpu.VMEM
    scratch = [
        vm((D, D), BF), vm((D, D), BF), vm((D, D), BF), vm((D, D), BF),
        vm((D, D), BF), vm((D, D), BF), vm((D, F), BF), vm((F, D), BF),
        vm((S, D), F32), vm((S, D), F32), vm((S + 2 * HPAD, D), F32),
        vm((S, D), BF), vm((S, D), BF),
        vm((L, D), BF), vm((L, D), BF), vm((L, D), BF), vm((L, D), BF),
        vm((NG, VR, L), BF), vm((L, D), BF),
        vm((2, NG, VR, 128), F32), vm((H, 128), F32), vm((2, 128, 128), F32),
        pltpu.SemaphoreType.DMA((9 + S // RB,)), pltpu.SemaphoreType.DMA((8,)),
        pltpu.SemaphoreType.DMA((NG // GPI, 3)),
    ]
    return pl.pallas_call(
        _kernel,
        out_shape=jax.ShapeDtypeStruct((1, S, D), BF),
        in_specs=[pl.BlockSpec(memory_space=pltpu.VMEM)] + [any_spec] * 9,
        out_specs=any_spec,
        scratch_shapes=scratch,
        compiler_params=pltpu.CompilerParams(vmem_limit_bytes=110 * 2 ** 20),
        name="fused_infini_mixer",
    )(A_beta.reshape(1, H), A_x, A_wq, A_wk, A_wv, A_wo, B_w1, B_w2, B_w3, B_w4)
```

```python
import numpy as np
import jax
import jax.numpy as jnp
from jax import lax
import jax.experimental.pallas as pl
import jax.experimental.pallas.tpu as pltpu

S, D, H, DH, NSEG, L, F = 2048, 1024, 32, 32, 4, 512, 3584
NG = D // 128
BF, F32 = jnp.bfloat16, jnp.float32
NT = (((1,), (1,)), ((), ()))
EPS = 1e-5
LOG2E = float(np.log2(np.e))
QSCALE = float(DH ** -0.5) * LOG2E
GC = float(np.sqrt(2.0 / np.pi))
HPAD = 8
L_LO, L_HI = 2.0 ** -40, 2.0 ** 40
MASKV = -1e9 * LOG2E
GPI = 4
LA = 2
LNG = 1
IORD = (0, 3, 2, 1)
RB = 256
PRB = 256
PCH, BCH = 128, 128
FC = 896
VR = 144


def _ln(x):
    m = jnp.mean(x, axis=-1, keepdims=True)
    xc = x - m
    v = jnp.mean(xc * xc, axis=-1, keepdims=True)
    return xc * lax.rsqrt(v + EPS)


def _gelu(x):
    return 0.5 * x * (1.0 + jnp.tanh(GC * (x + 0.044715 * (x * x * x))))


def _phi(x):
    return jnp.where(x > 0, x + 1.0, jnp.exp(x))


def _dot(a, b):
    return jnp.dot(a, b, preferred_element_type=F32)


def _dot_nt(a, b):
    return lax.dot_general(a, b, NT, preferred_element_type=F32)


def _head_mask(x, j):
    lane = lax.broadcasted_iota(jnp.int32, (1, 128), 1)
    m = jnp.where((lane >= 32 * j) & (lane < 32 * j + 32), -1, 0).astype(jnp.int32)
    return pltpu.bitcast(pltpu.bitcast(x, jnp.int32) & m, BF)


def _kernel(beta_ref, x_hbm, wq_hbm, wk_hbm, wv_hbm, wo_hbm, w1_hbm, w2_hbm, w3_hbm, w4_hbm,
            out_hbm,
            wq, wk, wv, wo, w1, w2, w3, w4,
            xf, xn_s, h_s, xio, xnb, qs, pq, ks, pk, vt, o_s, mst, gtab, mtab, sem, osem, qsem):
    def cp(src, dst, i):
        return pltpu.make_async_copy(src, dst, sem.at[i])
    NB = S // RB

    def c_xb(i):
        r = pl.multiple_of(i * RB, RB)
        return cp(x_hbm.at[0, pl.ds(r, RB)], xio.at[pl.ds(r, RB)], 9 + i)
    WC = GPI * 128

    def c_qkv(j):
        c = pl.multiple_of(j * WC, WC)
        return [pltpu.make_async_copy(src.at[:, pl.ds(c, WC)], dst.at[:, pl.ds(c, WC)], qsem.at[j, m])
                for m, (src, dst) in enumerate(((wv_hbm, wv), (wq_hbm, wq), (wk_hbm, wk)))]
    c_w = [cp(wo_hbm, wo, 4), cp(w1_hbm, w1, 5), cp(w2_hbm, w2, 6), cp(w3_hbm, w3, 7), cp(w4_hbm, w4, 8)]
    assert NG // GPI == 2 and L // RB == 2
    for c in [c_xb(0), c_xb(1), c_xb(2)] + c_qkv(0):
        c.start()

    b = beta_ref[...].astype(F32)
    hrow = lax.broadcasted_iota(jnp.int32, (H, H), 0)
    hcol = lax.broadcasted_iota(jnp.int32, (H, H), 1)
    bcol = jnp.sum(jnp.where(hrow == hcol, jnp.broadcast_to(b, (H, H)), 0.0), axis=1, keepdims=True)
    gtab[...] = jnp.broadcast_to(jax.nn.sigmoid(bcol), (H, 128))

    mr = lax.broadcasted_iota(jnp.int32, (128, 128), 0)
    mc = lax.broadcasted_iota(jnp.int32, (128, 128), 1)
    mtab[0] = jnp.where(mr <= (mc ^ 64), jnp.inf, 0.0)
    mtab[1] = jnp.where(mr <= mc, jnp.inf, 0.0)
    for g in range(NG):
        vt[g, 128:VR, :] = jnp.ones((VR - 128, L), BF)
    h_s[0:HPAD, :] = jnp.zeros((HPAD, D), F32)
    h_s[HPAD + S:HPAD + S + HPAD, :] = jnp.zeros((HPAD, D), F32)

    def cvt(i, c):
        c_xb(i).wait()
        r = pl.multiple_of(i * RB, RB)
        xf[pl.ds(r, RB), :] = xio[pl.ds(r, RB), :].astype(F32)
        return c
    lax.fori_loop(0, 2, cvt, 0)

    def attention_groups(g0, ngroups, par, bad, r0, rn):
        flag = [bad]
        steps = [(gg, i, t) for gg in range(ngroups) for i in IORD for t in range(i + 1)]
        ctx, wcache, state, mem = {}, {}, {}, {}

        xb = [xnb[pl.ds(r0, L), :]]

        def project(gg):
            g = g0 + gg
            c0 = pl.multiple_of(g * 128, 128)
            v = _dot(xb[0], wv[:, pl.ds(c0, 128)])
            vt[g, 0:128, :] = v.T.astype(BF)
            q = _dot(xb[0], wq[:, pl.ds(c0, 128)])
            qs[:, pl.ds(c0, 128)] = (q * QSCALE).astype(BF)
            pq[:, pl.ds(c0, 128)] = _phi(q).astype(BF)
            k = _dot(xb[0], wk[:, pl.ds(c0, 128)])
            ks[:, pl.ds(c0, 128)] = k.astype(BF)
            pk[:, pl.ds(c0, 128)] = _phi(k).astype(BF)
            if gg == LNG:
                xnb[pl.ds(rn, RB), :] = _ln(xf[pl.ds(rn, RB), :]).astype(BF)
                xb[0] = xnb[pl.ds(r0, L), :]

        def getg(gg):
            if gg not in ctx:
                g = g0 + gg
                c0 = pl.multiple_of(g * 128, 128)
                ctx[gg] = (g, c0, qs[:, pl.ds(c0, 128)], ks[:, pl.ds(c0, 128)], vt[g])
            return ctx[gg]

        def mem_read(gg):
            g, c0, _, _, vtg = getg(gg)
            nd = _dot_nt(mst[par, g].astype(BF), pq[:, pl.ds(c0, 128)])
            gates = [gtab[pl.ds(4 * g + j, 1), :] for j in range(4)]
            mem[gg] = (nd, gates)

        def mem_update(gg):
            g, c0, _, _, vtg = getg(gg)
            upd = _dot(vtg, pk[:, pl.ds(c0, 128)])
            r = lax.broadcasted_iota(jnp.int32, (VR, 128), 0)
            c = lax.broadcasted_iota(jnp.int32, (VR, 128), 1)
            keep = jnp.where(r < 128, r // 32, r - 128) == c // 32
            mst[1 - par, g] = mst[par, g] + jnp.where(keep, upd, 0.0)

        def qk(st):
            gg, i, t = st
            _, _, qg, kg, _ = getg(gg)
            if (gg, i) not in wcache:
                lo, hi = qg[128 * i:128 * i + 64], qg[128 * i + 64:128 * (i + 1)]
                ms = [_head_mask(jnp.concatenate([lo, hi] if j % 2 else [hi, lo], axis=0), j)
                      for j in range(4)]
                wcache[(gg, i)] = (jnp.concatenate(ms, axis=0),
                                   jnp.concatenate([ms[0][:64], ms[1][64:], ms[2][:64], ms[3][64:]], axis=0))
            W, Whi = wcache[(gg, i)]
            if t < i:
                return _dot_nt(kg[128 * t:128 * (t + 1)], W)
            return (_dot_nt(kg[128 * t:128 * t + 64], W),
                    _dot_nt(kg[128 * t + 64:128 * (t + 1)], Whi))

        def probs(St, j):
            if not isinstance(St, tuple):
                return jnp.exp2(St[:, 128 * j:128 * (j + 1)])
            Slo, Shi = St
            plo = jnp.minimum(jnp.exp2(Slo[:, 128 * j:128 * (j + 1)]), mtab[j % 2, 0:64])
            phi = jnp.minimum(Ehi[j // 2], mtab[j % 2, 64:128])
            return jnp.concatenate([plo, phi], axis=0)

        Ehi = [None, None]

        def softmax_tile(st, St):
            gg, i, t = st
            accs, ls = state.setdefault((gg, i), ([None] * 4, [None] * 4))
            if isinstance(St, tuple):
                Ehi[:] = [jnp.exp2(St[1][:, :128]), jnp.exp2(St[1][:, 128:])]
            out = []
            for j in range(4):
                P = probs(St, j)
                ps = jnp.sum(P.reshape(16, 8, 128), axis=0)
                ls[j] = ps if ls[j] is None else ls[j] + ps
                out.append(P.astype(BF))
            return out

        def pv(st, Pb):
            gg, i, t = st
            g, c0, _, _, vtg = getg(gg)
            accs, ls = state[(gg, i)]
            for j in range(4):
                O = _dot(vtg[32 * j:32 * j + 32, 128 * t:128 * (t + 1)], Pb[j])
                accs[j] = O if accs[j] is None else accs[j] + O
            if t == i:
                nd, gates = mem[gg]
                rows = []
                for j in range(4):
                    l = jnp.sum(ls[j], axis=0, keepdims=True)
                    flag[0] = jnp.where((l >= L_LO) & (l <= L_HI), flag[0], 1.0)
                    gj = gates[j]
                    den = nd[128 + j:129 + j, 128 * i:128 * (i + 1)] + 1e-6
                    num = nd[32 * j:32 * j + 32, 128 * i:128 * (i + 1)]
                    dot = accs[j] * ((1.0 - gj) / l)
                    if j % 2 == 0:
                        dot = pltpu.roll(dot, 64, 1)
                    rows.append(dot + num * (gj / den))
                o_s[128 * i:128 * (i + 1), pl.ds(c0, 128)] = jnp.concatenate(rows, axis=0).T.astype(BF)

        pend = []
        project(0)
        for n, st in enumerate(steps):
            gg, pos = divmod(n, 10)
            if pos == 0:
                if gg + 1 < ngroups:
                    project(gg + 1)
                mem_read(gg)
            pend.append((st, softmax_tile(st, qk(st))))
            if len(pend) > LA:
                pv(*pend.pop(0))
        upd = list(range(ngroups))
        while pend:
            mem_update(upd.pop(0))
            pv(*pend.pop(0))
        for gg in upd:
            mem_update(gg)
        return flag[0]

    def attention_safe(par):
        def body(n, c):
            g, i = n // 4, n % 4
            c0 = pl.multiple_of(g * 128, 128)
            q0 = pl.multiple_of(i * 128, 128)
            qi = qs[pl.ds(q0, 128), pl.ds(c0, 128)]
            W = jnp.concatenate([_head_mask(qi, j) for j in range(4)], axis=0)
            kr = lax.broadcasted_iota(jnp.int32, (128, 512), 0)
            qc = lax.broadcasted_iota(jnp.int32, (128, 512), 1) & 127

            def logits(t):
                k0 = pl.multiple_of(t * 128, 128)
                St = _dot_nt(ks[pl.ds(k0, 128), pl.ds(c0, 128)], W)
                return St + jnp.where(kr + k0 > qc + q0, MASKV, 0.0), k0

            def pass1(t, m):
                return jnp.maximum(m, jnp.max(logits(t)[0], axis=0, keepdims=True))
            m = lax.fori_loop(0, i + 1, pass1, jnp.full((1, 512), -jnp.inf, F32))

            def pass2(t, carry):
                acc, l = carry
                St, k0 = logits(t)
                P = jnp.exp2(St - m)
                outs = [_dot(vt[g, 32 * j:32 * j + 32, pl.ds(k0, 128)],
                             P[:, 128 * j:128 * (j + 1)].astype(BF)) for j in range(4)]
                return acc + jnp.concatenate(outs, axis=0), l + jnp.sum(P, axis=0, keepdims=True)
            acc, l = lax.fori_loop(0, i + 1, pass2,
                                   (jnp.zeros((128, 128), F32), jnp.zeros((1, 512), F32)))

            nd = _dot_nt(mst[par, g].astype(BF), pq[pl.ds(q0, 128), pl.ds(c0, 128)])
            rows = []
            for j in range(4):
                gj = gtab[pl.ds(4 * g + j, 1), :]
                den = nd[128 + j:129 + j, :] + 1e-6
                rows.append(acc[32 * j:32 * j + 32] * ((1.0 - gj) / l[:, 128 * j:128 * (j + 1)])
                            + nd[32 * j:32 * j + 32] * (gj / den))
            o_s[pl.ds(q0, 128), pl.ds(c0, 128)] = jnp.concatenate(rows, axis=0).T.astype(BF)
            return c
        lax.fori_loop(0, NG * 4, body, 0)

    def layer(ell, carry):
        mst[0] = jnp.zeros((NG, VR, 128), F32)

        def ln0(i, c):
            r = pl.multiple_of(i * RB, RB)
            xnb[pl.ds(r, RB), :] = _ln(xf[pl.ds(r, RB), :]).astype(BF)
            return c
        lax.fori_loop(0, L // RB, ln0, 0)

        def seg(s, c):
            r0 = pl.multiple_of(s * L, L)
            par = s % 2

            def qa(j, bad):
                nb = (s + 1) * (L // RB) + j

                @pl.when(ell == 0)
                def _():
                    @pl.when(nb < NB)
                    def _():
                        cvt(nb, 0)

                    @pl.when(s == 0)
                    def _():
                        for cw in c_qkv(j):
                            cw.wait()

                        @pl.when(j == 0)
                        def _():
                            for cw in [c_xb(3)] + c_qkv(1):
                                cw.start()

                        @pl.when(j == 1)
                        def _():
                            for cw in c_w[:2] + [c_xb(i) for i in range(4, NB)]:
                                cw.start()
                rn = pl.multiple_of(jnp.minimum(nb, NB - 1) * RB, RB)
                return attention_groups(j * GPI, GPI, par, bad, r0, rn)
            bad = lax.fori_loop(0, NG // GPI, qa, jnp.zeros((1, 128), F32))

            @pl.when(jnp.max(bad) > 0.0)
            def _():
                attention_safe(par)

            @pl.when(jnp.logical_and(ell == 0, s == 0))
            def _():
                for cw in c_w[:2]:
                    cw.wait()
                for cw in c_w[2:]:
                    cw.start()

            def proj(u, c3):
                offs = [pl.multiple_of(u * PRB + ch * PCH, PCH) for ch in range(PRB // PCH)]
                xs = []
                for o in offs:
                    x = xf[pl.ds(r0 + o, PCH), :] + _dot(o_s[pl.ds(o, PCH), :], wo[...])
                    xf[pl.ds(r0 + o, PCH), :] = x
                    xs.append(x)
                for o, x in zip(offs, xs):
                    xn = _ln(x)
                    xn_s[pl.ds(r0 + o, PCH), :] = xn
                    h_s[pl.ds(pl.multiple_of(r0 + o + HPAD, 8), PCH), :] = _gelu(_dot(_ln(xn).astype(BF), w1[...]))
                return c3
            lax.fori_loop(0, L // PRB, proj, 0)
            return c
        lax.fori_loop(0, NSEG, seg, 0)

        @pl.when(ell == 0)
        def _():
            for cw in c_w[2:]:
                cw.wait()

        def blk(s, c):
            r0 = pl.multiple_of(s * RB, RB)
            offs = [pl.multiple_of(r0 + ch * BCH, BCH) for ch in range(RB // BCH)]
            c4 = D // 4
            hss = []
            for rr in offs:
                parts = []
                for ci, sh in enumerate((-1, 1, -2, 2)):
                    w0 = rr if sh < 0 else rr + HPAD
                    win = h_s[pl.ds(pl.multiple_of(w0, 8), BCH + HPAD), ci * c4:(ci + 1) * c4]
                    o0 = HPAD + sh if sh < 0 else sh
                    parts.append(win[o0:o0 + BCH].astype(BF))
                hss.append(_dot(jnp.concatenate(parts, axis=1), w2[...]))
            for rr, hs in zip(offs, hss):
                x1 = xn_s[pl.ds(rr, BCH), :] + hs
                x1n = _ln(x1).astype(BF)
                acc = xf[pl.ds(rr, BCH), :] + x1
                for f in range(F // FC):
                    hh = _gelu(_dot(x1n, w3[:, f * FC:(f + 1) * FC])).astype(BF)
                    acc = acc + _dot(hh, w4[f * FC:(f + 1) * FC, :])
                xf[pl.ds(rr, BCH), :] = acc
                xio[pl.ds(rr, BCH), :] = acc.astype(BF)

            @pl.when(ell == 1)
            def _():
                pltpu.make_async_copy(xio.at[pl.ds(r0, RB)], out_hbm.at[0, pl.ds(r0, RB)], osem.at[s]).start()
            return c
        lax.fori_loop(0, S // RB, blk, 0)
        return carry

    lax.fori_loop(0, 2, layer, 0)
    for s in range(S // RB):
        pltpu.make_async_copy(xio.at[pl.ds(s * RB, RB)], out_hbm.at[0, pl.ds(s * RB, RB)], osem.at[s]).wait()


@jax.jit
def pallas_interleave_layers__memory_aug_infini_attn__mixer_s_mlp__prompt_kernel(
    A_x, A_wq, A_wk, A_wv, A_wo, A_beta, B_x, B_w1, B_w2, B_w3, B_w4,
):
    del B_x
    any_spec = pl.BlockSpec(memory_space=pl.ANY)
    vm = pltpu.VMEM
    scratch = [
        vm((D, D), BF), vm((D, D), BF), vm((D, D), BF), vm((D, D), BF),
        vm((D, D), BF), vm((D, D), BF), vm((D, F), BF), vm((F, D), BF),
        vm((S, D), F32), vm((S, D), F32), vm((S + 2 * HPAD, D), F32),
        vm((S, D), BF), vm((S, D), BF),
        vm((L, D), BF), vm((L, D), BF), vm((L, D), BF), vm((L, D), BF),
        vm((NG, VR, L), BF), vm((L, D), BF),
        vm((2, NG, VR, 128), F32), vm((H, 128), F32), vm((2, 128, 128), F32),
        pltpu.SemaphoreType.DMA((9 + S // RB,)), pltpu.SemaphoreType.DMA((8,)),
        pltpu.SemaphoreType.DMA((NG // GPI, 3)),
    ]
    return pl.pallas_call(
        _kernel,
        out_shape=jax.ShapeDtypeStruct((1, S, D), BF),
        in_specs=[pl.BlockSpec(memory_space=pltpu.VMEM)] + [any_spec] * 9,
        out_specs=any_spec,
        scratch_shapes=scratch,
        compiler_params=pltpu.CompilerParams(vmem_limit_bytes=110 * 2 ** 20),
        name="fused_infini_mixer",
    )(A_beta.reshape(1, H), A_x, A_wq, A_wk, A_wv, A_wo, B_w1, B_w2, B_w3, B_w4)
```
